```python
import os as _os
_os.environ.setdefault("JAX_PLATFORMS", "cpu")
import jax
import jax.numpy as jnp

def _softmax(x, axis=-1):
    return jax.nn.softmax(x, axis=axis)
def _gelu(x):
    return jax.nn.gelu(x, approximate=True)
def _silu(x):
    return jax.nn.silu(x)
def _sigmoid(x):
    return jax.nn.sigmoid(x)
def _layernorm(x, axis=-1, eps=1e-5):
    m = jnp.mean(x, axis=axis, keepdims=True)
    v = jnp.var(x, axis=axis, keepdims=True)
    return (x - m) / jnp.sqrt(v + eps)
def _scatter_add(tgt, idx, src, axis=0):
    return tgt.at[idx].add(src)
def _segment_sum(src, seg, n):
    return jax.ops.segment_sum(src, seg, n)
class _Rng:
    def __init__(self, key):
        self._k = key
    def _next(self):
        self._k, sub = jax.random.split(self._k)
        return sub
    def normal(self, shape):
        return jax.random.normal(self._next(), shape, dtype=jnp.bfloat16)
    def randint(self, lo, hi, shape):
        return jax.random.randint(self._next(), shape, lo, hi, dtype=jnp.int32)
    def uniform(self, shape, lo=0.0, hi=1.0):
        return jax.random.uniform(self._next(), shape, jnp.bfloat16, lo, hi)
    def permutation(self, n):
        return jax.random.permutation(self._next(), n)


kernel_name = 'interleave_layers__ssm_conv_h3__linear_attn_block__prompt'

def setup_inputs():
    _rng = _Rng(jax.random.key(int.from_bytes(__import__("os").urandom(4), "little")))
    _w = (lambda a: (lambda t: t.astype(jnp.bfloat16) if jnp.issubdtype(t.dtype, jnp.floating) else t)(jnp.asarray(a)))
    def _A_setup():
        B, S, D = 1, 2048, 512
        ks = 4
        return {
            "q": _w((lambda *s: _rng.normal(s) * 0.05)(B, S, D)),
            "k": _w((lambda *s: _rng.normal(s) * 0.4)(B, S, D)),
            "v": _w((lambda *s: _rng.normal(s) * 0.4)(B, S, D)),
            "shift_k": _w((lambda *s: _rng.normal(s) * 0.4)(D, ks) * 0.5),
            "ssm_k": _w((lambda *s: _rng.normal(s) * 0.4)(D, S) * (1.0 / S ** 0.5)),
            "ssm_D": _w((lambda *s: _rng.normal(s) * 0.4)(D)),
        }
    _A_in = _A_setup()

    def _B_setup():
        B, S, D = 1, 2048, 512
        return {
            "x": _w((lambda *s: _rng.normal(s) * 0.05)(B, S, D)),
            "wqkv": _w((lambda *s: _rng.normal(s) * 0.1)(D, 3 * D)),
            "wo": _w((lambda *s: _rng.normal(s) * 0.1)(D, D)),
        }
    _B_in = _B_setup()

    return {
        "A_q": _A_in["q"],
        "A_k": _A_in["k"],
        "A_v": _A_in["v"],
        "A_shift_k": _A_in["shift_k"],
        "A_ssm_k": _A_in["ssm_k"],
        "A_ssm_D": _A_in["ssm_D"],
        "B_x": _B_in["x"],
        "B_wqkv": _B_in["wqkv"],
        "B_wo": _B_in["wo"],
    }

def reference(A_q, A_k, A_v, A_shift_k, A_ssm_k, A_ssm_D, B_x, B_wqkv, B_wo):
    def _A_ref(q, k, v, shift_k, ssm_k, ssm_D):
        B, S, D = q.shape
        ks = shift_k.shape[-1]
        k_pad = jnp.pad(k, ((0, 0), (ks - 1, 0), (0, 0)))
        k_shift = jnp.zeros_like(k)
        for t in range(ks):
            k_shift = k_shift + k_pad[:, t:t + S, :] * shift_k[:, ks - 1 - t][None, None, :]
        kv = k_shift * v
        L = 2 * S
        kv_pad = jnp.pad(kv, ((0, 0), (0, S), (0, 0)))
        kf_pad = jnp.pad(ssm_k, ((0, 0), (0, S)))
        kv_f = (lambda x, axes=(-2,-1): jnp.fft.rfft2(x.astype(jnp.float32), axes=axes))(kv_pad[:, None, :, :], axes=(1, 2))
        kf_f = (lambda x, axes=(-2,-1): jnp.fft.rfft2(x.astype(jnp.float32), axes=axes))(kf_pad[:, None, :], axes=(1, 2))
        kf_f = (lambda x, *d: x.transpose(*d))(kf_f, 1, 2, 0)
        y_f = kv_f * kf_f[None, :, :, :]
        y = (lambda x, s, axes=(-2,-1): jnp.fft.irfft2(x, s=s, axes=axes).astype(jnp.bfloat16))(y_f, (1, L), axes=(1, 2))[:, 0, :S, :]
        y = y + kv * ssm_D[None, None, :]
        return q * y

    def _B_ref(x, wqkv, wo):
        B, S, D = x.shape
        H = 32; Dh = D // H
        qkv = (lambda x, *d: x.transpose(*d))((x @ wqkv).reshape(B, S, 3, H, Dh), 2, 0, 3, 1, 4)
        q, k, v = qkv[0], qkv[1], qkv[2]
        phi = lambda t: jnp.where(t > 0, t + 1, jnp.exp(t)) + 1e-6
        pq, pk = phi(q), phi(k)
        kv = jnp.einsum("bhsd,bhse->bhde", pk, v)
        z = jnp.einsum("bhsd->bhd", pk)
        num = jnp.einsum("bhqd,bhde->bhqe", pq, kv)
        den = jnp.einsum("bhqd,bhd->bhq", pq, z)[..., None] + 1e-6
        o = num / den
        return (lambda x, *d: x.transpose(*d))(o, 0, 2, 1, 3).reshape(B, S, D) @ wo

    x = A_q
    x = x + _A_ref(_layernorm(x, axis=-1), A_k, A_v, A_shift_k, A_ssm_k, A_ssm_D)
    x = x + _B_ref(_layernorm(x, axis=-1), B_wqkv, B_wo)
    x = x + _A_ref(_layernorm(x, axis=-1), A_k, A_v, A_shift_k, A_ssm_k, A_ssm_D)
    x = x + _B_ref(_layernorm(x, axis=-1), B_wqkv, B_wo)
    return x
```

```python
import numpy as np
import jax
import jax.numpy as jnp
from jax import lax
import jax.experimental.pallas as pl
import jax.experimental.pallas.tpu as pltpu

S, D = 2048, 512
T = 128
NB = S // T
NG = 4
SB = S // NG
NT = D // 128
DH = 16
HALO = 16
EPS_LN = 1e-5
RC = 32
LSTEP = 16
LAT_M = 200.0
LAT_X = 80.0
VR = 3.5
SLACK_M = 256.0
PACE = 0.8
HUNGRY = 32.0
GALL = 1
LAGM = 0.0
GV = 0
LAG = -1.0
PH2 = 3
F32 = jnp.float32
BF16 = jnp.bfloat16
U32 = jnp.uint32


def _pack_rows_np(a):
    u = np.ascontiguousarray(a, np.float32).view(np.uint32)
    b = ((u + 0x7FFF + ((u >> 16) & 1)) >> 16).astype(np.uint32)
    return (b[0::2] | (b[1::2] << 16)).astype(np.uint32)


def _dft_mats():
    N = 2 * T
    ks = np.concatenate([np.arange(0, T, 2), np.arange(1, T, 2)])
    n = np.arange(T)
    th = np.pi * np.outer(2 * ks + 1, n) / N
    c_, s_ = np.cos(th), -np.sin(th)
    F = np.stack([c_.reshape(T // 8, 8, T), s_.reshape(T // 8, 8, T)], 1).reshape(2 * T, T)
    Gr = np.cos(th).T * (2.0 / N)
    Gi = -np.sin(th).T * (2.0 / N)
    G = np.stack([Gr.reshape(T, T // 8, 8), Gi.reshape(T, T // 8, 8)], 2).reshape(T, 2 * T)
    return _pack_rows_np(F), _pack_rows_np(G)


def _bf(u):
    return pltpu.bitcast(u, BF16)


def _pk(x):
    return pltpu.bitcast(x.astype(BF16), U32)


def _stats(x):
    m = jnp.sum(x, axis=-1, keepdims=True) * (1.0 / D)
    e2 = jnp.sum(x * x, axis=-1, keepdims=True) * (1.0 / D)
    return m, lax.rsqrt(jnp.maximum(e2 - m * m, 0.0) + EPS_LN)


def _phi(t):
    return jnp.where(t > 0, t + (1.0 + 1e-6), jnp.exp(t) + 1e-6)


def _nt(a, b):
    return lax.dot_general(a, b, (((1,), (1,)), ((), ())), preferred_element_type=F32)


def _nn(a, b):
    return jnp.dot(a, b, preferred_element_type=F32)


def _mo(x, n):
    return x if isinstance(x, int) else pl.multiple_of(x, n)


def _gate(x, tok):
    if tok is None:
        return x
    dt = x.dtype
    u = x if dt == U32 else pltpu.bitcast(x, U32)
    r, c = u.shape
    top = u[0:8, 0:128] | tok
    if c > 128:
        top = jnp.concatenate([top, u[0:8, 128:]], axis=1)
    if r > 8:
        top = jnp.concatenate([top, u[8:]], axis=0)
    return top if dt == U32 else pltpu.bitcast(top, dt)


class Item:
    __slots__ = ('m', 'v', 'lat', 'fn', 'pri', 'after')

    def __init__(self, m, v, lat, fn, pri=2, after=None):
        self.m, self.v, self.lat, self.fn, self.pri, self.after = m, v, lat, fn, pri, after


def _merge(*streams, paced=()):
    st = [dict(items=list(s_), i=0, ready=0.0) for s_ in streams]
    tot_m = sum(it.m for s in st for it in s['items'])
    tot_v = sum(it.v for s in st for it in s['items']) / VR
    chain = max(sum(max(it.m, it.v / VR) + it.lat for it in s['items']) for s in st)
    horizon = max(tot_m, tot_v, chain) * PACE
    tm = tv = 0.0
    toks = []
    while True:
        live = [s for s in st if s['i'] < len(s['items'])]
        if not live:
            break
        head = lambda s: s['items'][s['i']]
        free = [s for s in live if head(s).after is None or st[head(s).after]['i'] >= len(st[head(s).after]['items'])]

        def earliest(s):
            t = s['ready']
            if head(s).m > 0:
                t = max(t, tm - SLACK_M)
            k = st.index(s)
            if k in paced:
                t = max(t, horizon * s['i'] / len(s['items']))
            return t
        ok = [s for s in free if earliest(s) <= tv]
        if ok:
            hungry = tm <= tv + HUNGRY
            s = max(ok, key=lambda s: ((head(s).m > 0) if hungry else 0, head(s).pri))
        else:
            s = min(free, key=earliest)
            tv = max(tv, min(earliest(s), max(s['ready'], tm - SLACK_M)))
        it = head(s)
        s['i'] += 1
        tin = None
        if it.m == 0 and LAG >= 0 and (it.pri == 1 or GV):
            cand = [tk for (tdone, tk, ism) in toks if ism and tdone + LAG <= tv]
            tin = cand[-1] if cand else None
        elif it.m > 0 and LAGM >= 0:
            cand = [tk for (tdone, tk, ism) in toks if not ism and tdone + LAGM <= max(tv, tm)]
            tin = cand[-1] if cand else None
        tout = it.fn(tin)
        if tout is not None:
            if it.m > 0:
                toks.append((max(tm, tv) + it.m, tout, True))
            else:
                prev = [tk for (_, tk, ism) in toks if not ism]
                if prev:
                    tout = tout | prev[-1]
                toks.append((tv + it.v / VR, tout, False))
        t0 = tv
        tv += it.v / VR
        end = tv
        if it.m > 0:
            tm = max(tm, t0) + it.m
            end = max(tm, tv) if it.lat else tv
        s['ready'] = end + it.lat


def kernel(z_ref, q_hbm, k_hbm, v_hbm, sk_ref, h_hbm, dd_ref, wqkv_hbm, wo_hbm, f_ref, g_ref,
           o_hbm,
           qb, kb, vb, hb, wqkv, wo, wqp, wktp, KF, KV,
           U0, U1, U2, U3, H0, H1, H2, H3, RA, ZSa, ZSb, Y, X1, X3, Q1, Q2,
           XNa, XNb, PKa, PKb, PNa, PNb, Oa, Ob, P, ZP, Mp, Zm, ob, sems, osems, sem0):

    def cp_k(g): return pltpu.make_async_copy(k_hbm.at[pl.ds(g * SB, SB)], kb.at[pl.ds(HALO + g * SB, SB)], sems.at[g])
    def cp_v(g): return pltpu.make_async_copy(v_hbm.at[pl.ds(g * SB, SB)], vb.at[pl.ds(g * SB, SB)], sems.at[4 + g])
    def cp_h(g): return pltpu.make_async_copy(h_hbm.at[:, pl.ds(g * SB, SB)], hb.at[:, pl.ds(g * SB, SB)], sems.at[8 + g])
    def cp_q(g): return pltpu.make_async_copy(q_hbm.at[pl.ds(g * SB, SB)], qb.at[pl.ds(g * SB, SB)], sems.at[12 + g])
    cp_w = pltpu.make_async_copy(wqkv_hbm.at[:, pl.ds(0, 2 * D)], wqkv.at[:, pl.ds(0, 2 * D)], sems.at[16])
    cp_wv = pltpu.make_async_copy(wqkv_hbm.at[:, pl.ds(2 * D, D)], wqkv.at[:, pl.ds(2 * D, D)], sems.at[18])
    cp_o = pltpu.make_async_copy(wo_hbm, wo, sems.at[17])

    def cp0(j):
        cs = pl.ds(_mo(j * 128, 128), 128)
        return (pltpu.make_async_copy(h_hbm.at[cs, pl.ds(0, SB)], hb.at[cs, pl.ds(0, SB)], sem0.at[0, j]),
                pltpu.make_async_copy(k_hbm.at[pl.ds(0, SB), cs], kb.at[pl.ds(HALO, SB), cs], sem0.at[1, j]),
                pltpu.make_async_copy(v_hbm.at[pl.ds(0, SB), cs], vb.at[pl.ds(0, SB), cs], sem0.at[2, j]))

    for j in range(NT):
        for c in cp0(j):
            c.start()
    cp_h(1).start(); cp_k(1).start(); cp_v(1).start()
    cp_w.start()
    for g in range(2, NG):
        cp_q(g - 2).start(); cp_h(g).start(); cp_k(g).start(); cp_v(g).start()
    cp_q(2).start(); cp_q(3).start(); cp_wv.start(); cp_o.start()

    kb[pl.ds(0, HALO), :] = jnp.zeros((HALO, D), BF16)
    P[...] = jnp.zeros(P.shape, F32)
    ZP[...] = jnp.zeros(ZP.shape, F32)
    XNa[...] = jnp.zeros(XNa.shape, U32)

    h2 = T // 2
    zi = z_ref[0]
    zm = jnp.full((8, 128), zi, jnp.int32).astype(U32)

    def tokof(x):
        u = x if x.dtype == U32 else pltpu.bitcast(x, U32)
        return u[-8:, -128:] & zm

    def tokst(r):
        u = pltpu.bitcast(jnp.broadcast_to(r, (r.shape[0], 128)), U32)
        t = u[0:8]
        for k in range(1, r.shape[0] // 8):
            t = t | u[8 * k:8 * k + 8]
        return t & zm

    XN = (XNa, XNb); PK = (PKa, PKb); PN = (PNa, PNb); OO = (Oa, Ob)
    UC = (U0, U1, U2, U3); HC = (H0, H1, H2, H3); ZS = (ZSa, ZSb)

    def pre_items(g, j):
        cs = pl.ds(_mo(j * 128, 128), 128)
        items = []

        def spec_store(dst, i, val, e, is_h):
            for gi in range(8):
                re = val[16 * gi:16 * gi + 8]
                im = val[16 * gi + 8:16 * gi + 16]
                rs = pl.ds(e * h2 + 8 * gi, 8)
                if is_h:
                    if g == 0 and i == 0:
                        re = re + dd_ref[:, cs].astype(F32)
                    dst[j, i, 0, rs, :] = re + im
                    dst[j, i, 1, rs, :] = re
                    dst[j, i, 2, rs, :] = im
                else:
                    dst[j, i, 0, rs, :] = re
                    dst[j, i, 1, rs, :] = im - re
                    dst[j, i, 2, rs, :] = re + im

        def a_dot(i, e):
            def fn(tok):
                a_ = _nt(_bf(_gate(f_ref[e * 64:(e + 1) * 64, :], tok)), hb[cs, pl.ds((4 * g + i) * T, T)])
                spec_store(HC[g], i, a_, e, True)
                return tokof(a_)
            return Item(32, 20, 0, fn, 3)

        def kf(i):
            def fn(tok):
                n = T + (HALO if i == 0 else 0)
                o = 0 if i == 0 else HALO + i * T
                KF[0, o:o + n, :] = kb[pl.ds(g * SB + o, n), cs].astype(F32)
            return Item(0, 20, 0, fn, 3)

        def shift(i, hf):
            def fn(tok):
                sk = sk_ref[:, cs].astype(F32)
                o = HALO + i * T + hf * h2
                ks = _gate(KF[zi, o:o + h2, :], tok) * sk[0:1]
                for s in range(1, 4):
                    ks = ks + KF[zi, o - s:o - s + h2, :] * sk[s:s + 1]
                kv = _pk(ks * vb[pl.ds((4 * g + i) * T + hf * h2, h2), cs].astype(F32))
                KV[i, hf * 32:(hf + 1) * 32, :] = kv
                return tokof(kv)
            return Item(0, 80, 0, fn, 3)

        def u_dot(i, e):
            def fn(tok):
                u = _nn(_bf(_gate(f_ref[e * 64:(e + 1) * 64, :], tok)), _bf(KV[i + zi]))
                spec_store(UC[g], i, u, e, False)
                return tokof(u)
            return Item(32, 16, 0, fn, 3)

        items += [a_dot(0, 0), a_dot(0, 1)]
        for i in range(4):
            items += [kf(i), shift(i, 0), shift(i, 1)]
            if i < 3:
                items += [a_dot(i + 1, 0), a_dot(i + 1, 1)]
            items += [u_dot(i, 0), u_dot(i, 1)]
        return items

    def mac_items(g, j):
        items = []
        state = {}
        zs = ZS[g % 2]

        def mac(fi, l0, l1, last):
            fs = pl.ds(fi * 8, 8)
            n = sum(1 for l in range(l0, l1) for o in range(4) if 4 * g + o - l >= 0)

            def fn(tok):
                if l0 == 0:
                    state['acc'] = [[None] * 3 for _ in range(4)]
                acc = state['acc']
                for l in range(l0, l1):
                    h = [HC[l // 4][j, l % 4, c, fs, :] for c in range(3)]
                    if l == l0 or GALL:
                        h = [_gate(x, tok) for x in h]
                    for o in range(4):
                        m = 4 * g + o - l
                        if m < 0:
                            continue
                        for c in range(3):
                            t = h[c] * UC[m // 4][j, m % 4, c, fs, :]
                            acc[o][c] = t if acc[o][c] is None else acc[o][c] + t
                if last:
                    yr = [acc[o][0] - acc[o][2] for o in range(4)]
                    yi = [acc[o][0] + acc[o][1] for o in range(4)]
                    for o in range(4):
                        if o == 0 and g == 0:
                            zr, zi_ = yr[0], yi[0]
                        else:
                            pr, pi = (RA[j, 0, fs, :], RA[j, 1, fs, :]) if o == 0 else (yr[o - 1], yi[o - 1])
                            if fi < 8:
                                zr, zi_ = yr[o] - pi, yi[o] + pr
                            else:
                                zr, zi_ = yr[o] + pi, yi[o] - pr
                        zp_ = _pk(jnp.concatenate([zr, zi_], axis=0))
                        zs[j, fs, o * 128:(o + 1) * 128] = zp_
                        allz = zp_ if o == 0 else allz | zp_
                    if g < NG - 1:
                        RA[j, 0, fs, :] = yr[3]
                        RA[j, 1, fs, :] = yi[3]
                return tokof(allz) if last else None
            return Item(0, 6 * n + (20 if last else 0), 0, fn, 1)

        nl = 4 * g + 4
        for fi in range(T // 8):
            for l0 in range(0, nl, LSTEP):
                l1 = min(nl, l0 + LSTEP)
                items.append(mac(fi, l0, l1, l1 == nl))
        return items

    def inv_items(g, j):
        cs = pl.ds(_mo(j * 128, 128), 128)

        def inv(i):
            def fn(tok):
                y = _nn(_bf(_gate(g_ref[...], tok)), _bf(ZS[g % 2][j + zi, :, i * 128:(i + 1) * 128]))
                Y[pl.ds((4 * g + i) * T, T), cs] = y
                return tokof(y)
            return Item(64, 16, 0, fn, 3)
        return [inv(i) for i in range(4)]

    def proj_items(r, Qo, par):
        xn, pkt = XN[par], PK[par]
        r0h = _mo(r * 64, 64)
        items = []

        def kdot(n):
            def fn(tok):
                pk = _phi(_nt(_bf(_gate(wktp[n * 64:(n + 1) * 64, :], tok)), _bf(xn[zi])))
                ZP[n * 128:(n + 1) * 128, :] += pk
                pkt[0, n * 64:(n + 1) * 64, :] = _pk(pk)
                return tokof(pk)
            return Item(128, 160, 0, fn)

        def qdot(n):
            def fn(tok):
                ns = slice(n * 128, (n + 1) * 128)
                q = _nn(_bf(_gate(xn[zi], tok)), _bf(wqp[:, ns]))
                Qo[pl.ds(r0h, 64), ns] = _pk(q)
                return tokof(q)
            return Item(128, 56, 0, fn)

        def pdot(n):
            def fn(tok):
                ds_ = slice(n * 128, (n + 1) * 128)
                p = _nn(_bf(_gate(pkt[zi, n * 64:(n + 1) * 64, :], tok)), _bf(xn[zi]))
                P[ds_, :] += p
                return tokof(p)
            return Item(128, 64, 0, fn)
        return [kdot(n) for n in range(4)] + [qdot(n) for n in range(4)] + [pdot(n) for n in range(4)]

    def ln_items(r, get_x, Xo, par):
        nc = T // RC
        st = {}
        vsc = RC / 32

        def rows(c):
            return pl.ds(_mo(r * T + c * RC, RC), RC)

        def rowsz(c):
            return pl.ds(pl.multiple_of(r * T + (c + zi) * RC, RC), RC)

        def sa(c):
            def fn(tok):
                st['a', c] = _stats(_gate(get_x(c, rows(c)), tok))
                return tokst(st['a', c][1])
            return Item(0, 90 * vsc, LAT_X if c == nc - 1 else 0, fn, 2.5)

        def sb(c):
            def fn(tok):
                m, rs_ = st['a', c]
                x = _gate(get_x(c, rows(c)), tok)
                x1 = x + (x - m) * rs_ * Y[rows(c), :]
                Xo[rows(c), :] = x1
                st['b', c] = _stats(x1)
                return tokst(st['b', c][1])
            return Item(0, 150 * vsc, LAT_X if c == nc - 1 else 0, fn, 2.5)

        def sc(c):
            def fn(tok):
                m, rs_ = st['b', c]
                xn = _pk((_gate(Xo[rowsz(c), :], tok) - m) * rs_)
                XN[par][0, c * RC // 2:(c + 1) * RC // 2, :] = xn
                return tokof(xn)
            return Item(0, 45 * vsc, 0, fn, 2.5)
        return [f(c) for f in (sa, sb) for c in range(nc)], [sc(c) for c in range(nc)]

    def d1_streams(r):
        ab, c_ = ln_items(r, lambda c, rs: qb[rs, :].astype(F32), X1, 0)
        for it in c_:
            it.after = 1
        return proj_items(jnp.maximum(r - 1, 0), Q1, 0) + c_, ab

    def wprep_items(n):
        ns = pl.ds(_mo(n * 128, 128), 128)

        def f1(tok):
            wqp[:, ns] = pltpu.bitcast(wqkv[:, ns], U32)

        def f2(tok):
            wktp[pl.ds(_mo(n * 64, 64), 64), :] = pltpu.bitcast(wqkv[:, pl.ds(_mo(D + n * 128, 128), 128)].T, U32)
        return [Item(0, 40, 0, f1), Item(0, 200, 0, f2)]

    rr = lax.broadcasted_iota(jnp.int32, (128, 128), 0) // DH
    cc = lax.broadcasted_iota(jnp.int32, (128, 128), 1) // DH
    mask = rr == cc

    def finish():
        z = jnp.sum(ZP[...], axis=-1, keepdims=True)
        kvs = []
        for g in range(4):
            sl = slice(g * 128, (g + 1) * 128)
            kvg = _nn(P[sl, :].astype(BF16), wqkv[:, 2 * D + g * 128:2 * D + (g + 1) * 128])
            kvs.append(jnp.where(mask, kvg, 0.0).astype(BF16))
        for g in range(4):
            sl = slice(g * 128, (g + 1) * 128)
            Zm[g] = _pk(jnp.where(mask, jnp.broadcast_to(z[sl], (128, 128)), 0.0))
            Mp[g * 64:(g + 1) * 64, :] = _pk(_nn(kvs[g], wo[sl, :]))
        P[...] = jnp.zeros(P.shape, F32)
        ZP[...] = jnp.zeros(ZP.shape, F32)

    def attn_items(r, Qi, par, sink):
        r0h = _mo(r * 64, 64)
        pn = PN[par]

        def e1(g):
            def fn(tok):
                sl = slice(g * 128, (g + 1) * 128)
                pq = _phi(_bf(_gate(Qi[pl.ds(r0h, 64), sl], tok)).astype(F32))
                den = _nn(pq.astype(BF16), _bf(Zm[g])) + 1e-6
                x = _pk(pq * pl.reciprocal(den, approx=True))
                pn[0, :, sl] = x
                return tokof(x)
            return Item(32, 150, LAT_M if g == 3 else 0, fn, 3)

        def e3(n, lat):
            def fn(tok):
                ns = slice(n * 128, (n + 1) * 128)
                o = _nn(_bf(_gate(pn[zi], tok)), _bf(Mp[:, ns]))
                sink(n, o)
                return tokof(o)
            return Item(128, 70, lat, fn, 3)
        return [e1(g) for g in range(4)] + [e3(n, LAT_M if n == 3 else 0) for n in range(4)]

    def att2_items(r, par):
        oo = OO[par]

        def sink(n, val):
            ns = slice(n * 128, (n + 1) * 128)
            oo[0, :, ns] = val + X1[pl.ds(_mo(r * T, T), T), ns]
        return attn_items(r, Q1, par, sink)

    def ln2_items(r, par):
        oo = OO[par]
        ab, c_ = ln_items(r, lambda c, rs: oo[zi, c * RC:(c + 1) * RC, :], X3, par)
        return ab + c_

    def ocp(i):
        r0 = pl.multiple_of(i * T, T)
        return pltpu.make_async_copy(ob.at[pl.ds(r0, T)], o_hbm.at[pl.ds(r0, T)], osems.at[i])

    def s3_items(r, par):
        r0 = pl.multiple_of(r * T, T)

        def sink(n, val):
            ns = slice(n * 128, (n + 1) * 128)
            ob[pl.ds(r0, T), ns] = (val + X3[pl.ds(r0, T), ns]).astype(BF16)
        return attn_items(r, Q2, par, sink)

    def bpre(j, _):
        for c in cp0(j):
            c.wait()
        _merge(pre_items(0, j))
        return 0
    lax.fori_loop(0, NT, bpre, 0)

    for g in range(NG + 1):
        if g + 1 < NG:
            cp_h(g + 1).wait(); cp_k(g + 1).wait(); cp_v(g + 1).wait()
        if g == 0:
            cp_w.wait()
        if g >= 1:
            cp_q(g - 1).wait()

        def bg(j, _, g=g):
            streams = []
            paced = ()
            if g >= 1:
                streams += list(d1_streams(4 * (g - 1) + j))
                paced = (0,)
            if g + 1 < NG:
                streams.append(pre_items(g + 1, j))
            if g == 0:
                streams.append(wprep_items(j))
            if g < NG:
                streams.append(mac_items(g, j) + inv_items(g, j))
            _merge(*streams, paced=paced)
            if g == 1:
                @pl.when(j == 0)
                def _():
                    P[...] = jnp.zeros(P.shape, F32)
                    ZP[...] = jnp.zeros(ZP.shape, F32)
            return 0
        lax.fori_loop(0, NT, bg, 0)
    _merge(proj_items(NB - 1, Q1, 0))
    cp_wv.wait()
    cp_o.wait()
    finish()

    if PH2 == 2:
        _merge(att2_items(0, 0) + ln2_items(0, 0))

        def ph2(i, _):
            a = 2 * i
            _merge(proj_items(a, Q2, 0), att2_items(a + 1, 1) + ln2_items(a + 1, 1), paced=(0,))
            nx = jnp.minimum(a + 2, NB - 1)
            _merge(proj_items(a + 1, Q2, 1), att2_items(nx, 0) + ln2_items(nx, 0), paced=(0,))
            return 0
        lax.fori_loop(0, NB // 2, ph2, 0)
    else:
        _merge(att2_items(0, 0))
        _merge(ln2_items(0, 0), att2_items(1, 1))

        def ph2(i, _):
            a = 2 * i
            c = lambda x: jnp.minimum(x, NB - 1)
            _merge(proj_items(a, Q2, 0), ln2_items(a + 1, 1), att2_items(c(a + 2), 0), paced=(0,))
            _merge(proj_items(a + 1, Q2, 1), ln2_items(c(a + 2), 0), att2_items(c(a + 3), 1), paced=(0,))
            return 0
        lax.fori_loop(0, NB // 2, ph2, 0)
    finish()

    def ph3(i, _):
        _merge(s3_items(2 * i, 0), s3_items(2 * i + 1, 1))
        ocp(2 * i).start()
        ocp(2 * i + 1).start()
        return 0
    lax.fori_loop(0, NB // 2, ph3, 0)

    def wt(i, _):
        ocp(i).wait()
        return 0
    lax.fori_loop(0, NB, wt, 0)


@jax.jit
def pallas_interleave_layers__ssm_conv_h3__linear_attn_block__prompt_kernel(A_q, A_k, A_v, A_shift_k, A_ssm_k, A_ssm_D, B_x, B_wqkv, B_wo):
    Fp, Gp = _dft_mats()
    anyspec = pl.BlockSpec(memory_space=pl.ANY)
    vspec = pl.BlockSpec(memory_space=pltpu.VMEM)
    half = lambda r, c: pltpu.VMEM((r // 2, c), U32)
    half1 = lambda r, c: pltpu.VMEM((1, r // 2, c), U32)
    spec = pltpu.VMEM((NT, 4, 3, T, 128), F32)
    out = pl.pallas_call(
        kernel,
        out_shape=jax.ShapeDtypeStruct((S, D), BF16),
        in_specs=[pl.BlockSpec(memory_space=pltpu.SMEM), anyspec, anyspec, anyspec, vspec, anyspec, vspec, anyspec, anyspec, vspec, vspec],
        out_specs=anyspec,
        scratch_shapes=[
            pltpu.VMEM((S, D), BF16),
            pltpu.VMEM((S + HALO, D), BF16),
            pltpu.VMEM((S, D), BF16),
            pltpu.VMEM((D, S), BF16),
            pltpu.VMEM((D, 3 * D), BF16),
            pltpu.VMEM((D, D), BF16),
            half(D, D),
            half(D, D),
            pltpu.VMEM((1, SB + HALO, 128), F32),
            pltpu.VMEM((4, T // 2, 128), U32),
            spec, spec, spec, spec,
            spec, spec, spec, spec,
            pltpu.VMEM((NT, 2, T, 128), F32),
            pltpu.VMEM((NT, T, D), U32),
            pltpu.VMEM((NT, T, D), U32),
            pltpu.VMEM((S, D), F32),
            pltpu.VMEM((S, D), F32),
            pltpu.VMEM((S, D), F32),
            half(S, D), half(S, D),
            half1(T, D), half1(T, D),
            half1(D, T), half1(D, T),
            half1(T, D), half1(T, D),
            pltpu.VMEM((1, T, D), F32), pltpu.VMEM((1, T, D), F32),
            pltpu.VMEM((D, D), F32),
            pltpu.VMEM((D, 128), F32),
            half(D, D),
            pltpu.VMEM((4, 64, 128), U32),
            pltpu.VMEM((S, D), BF16),
            pltpu.SemaphoreType.DMA((19,)),
            pltpu.SemaphoreType.DMA((NB,)),
            pltpu.SemaphoreType.DMA((3, NT)),
        ],
        compiler_params=pltpu.CompilerParams(vmem_limit_bytes=110 * 1024 * 1024),
    )(jnp.zeros((1,), jnp.int32), A_q.reshape(S, D), A_k.reshape(S, D), A_v.reshape(S, D), A_shift_k.T, A_ssm_k,
      A_ssm_D.reshape(1, D), B_wqkv, B_wo, jnp.asarray(Fp), jnp.asarray(Gp))
    return out.reshape(1, S, D)
```

```python
import numpy as np
import jax
import jax.numpy as jnp
from jax import lax
import jax.experimental.pallas as pl
import jax.experimental.pallas.tpu as pltpu

S, D = 2048, 512
T = 128
NB = S // T
NG = 4
SB = S // NG
NT = D // 128
DH = 16
HALO = 16
EPS_LN = 1e-5
RC = 32

LAT_M, LAT_X = 200.0, 80.0
VR = 4.0
SLACK_M, HUNGRY = 256.0, 32.0
LAGM, LAGX = 0.0, 200.0

F32 = jnp.float32
BF16 = jnp.bfloat16
U32 = jnp.uint32


def _pack_rows_np(a):
    u = np.ascontiguousarray(a, np.float32).view(np.uint32)
    b = ((u + 0x7FFF + ((u >> 16) & 1)) >> 16).astype(np.uint32)
    return (b[0::2] | (b[1::2] << 16)).astype(np.uint32)


def _dft_mats():
    n2 = 2 * T
    ks = np.concatenate([np.arange(0, T, 2), np.arange(1, T, 2)])
    th = np.pi * np.outer(2 * ks + 1, np.arange(T)) / n2
    c_, s_ = np.cos(th), -np.sin(th)
    fwd = np.stack([c_.reshape(T // 8, 8, T), s_.reshape(T // 8, 8, T)], 1).reshape(2 * T, T)
    inv = np.stack([c_.T.reshape(T, T // 8, 8), s_.T.reshape(T, T // 8, 8)], 2).reshape(T, 2 * T) * (2.0 / n2)
    return _pack_rows_np(fwd), _pack_rows_np(inv)


def _bf(u):
    return pltpu.bitcast(u, BF16)


def _pk(x):
    return pltpu.bitcast(x.astype(BF16), U32)


def _stats(x):
    m = jnp.sum(x, axis=-1, keepdims=True) * (1.0 / D)
    e2 = jnp.sum(x * x, axis=-1, keepdims=True) * (1.0 / D)
    return m, lax.rsqrt(jnp.maximum(e2 - m * m, 0.0) + EPS_LN)


def _phi(t):
    return jnp.where(t > 0, t + (1.0 + 1e-6), jnp.exp(t) + 1e-6)


def _nt(a, b):
    return lax.dot_general(a, b, (((1,), (1,)), ((), ())), preferred_element_type=F32)


def _nn(a, b):
    return jnp.dot(a, b, preferred_element_type=F32)


def _mo(x, n):
    return x if isinstance(x, int) else pl.multiple_of(x, n)


def _gate(u, tok):
    if tok is None:
        return u
    r, c = u.shape
    top = u[0:8, 0:128] | tok
    if c > 128:
        top = jnp.concatenate([top, u[0:8, 128:]], axis=1)
    if r > 8:
        top = jnp.concatenate([top, u[8:]], axis=0)
    return top


class Item:
    __slots__ = ('m', 'v', 'lat', 'fn', 'pri', 'after')

    def __init__(self, m, v, lat, fn, pri=2, after=None):
        self.m, self.v, self.lat, self.fn, self.pri, self.after = m, v, lat, fn, pri, after


def _merge(*streams, paced=(), pace=0.8, pin=False):
    st = [dict(items=list(s_), i=0, ready=0.0) for s_ in streams]
    tot_m = sum(it.m for s in st for it in s['items'])
    tot_v = sum(it.v for s in st for it in s['items']) / VR
    chain = max(sum(max(it.m, it.v / VR) + it.lat for it in s['items']) for s in st)
    horizon = max(tot_m, tot_v, chain) * pace
    tm = tv = 0.0
    toks = []
    head = lambda s: s['items'][s['i']]
    while True:
        live = [s for s in st if s['i'] < len(s['items'])]
        if not live:
            break
        free = [s for s in live if head(s).after is None or st[head(s).after]['i'] >= len(st[head(s).after]['items'])]

        def earliest(s):
            t = s['ready']
            if head(s).m > 0:
                t = max(t, tm - SLACK_M)
            if st.index(s) in paced:
                t = max(t, horizon * s['i'] / len(s['items']))
            return t
        ok = [s for s in free if earliest(s) <= tv]
        if ok:
            hungry = tm <= tv + HUNGRY
            s = max(ok, key=lambda s: ((head(s).m > 0) if hungry else 0, head(s).pri))
        else:
            s = min(free, key=earliest)
            tv = max(tv, min(earliest(s), max(s['ready'], tm - SLACK_M)))
        it = head(s)
        s['i'] += 1
        tin = None
        if it.m > 0 and pin:
            now = max(tv, tm)
            both = ([tk for (td, tk, k) in toks if k == 'v' and td + LAGM <= now][-1:]
                    + [tk for (td, tk, k) in toks if k == 'x' and td + LAGX <= now][-1:])
            tin = None if not both else (both[0] if len(both) == 1 else both[0] | both[1])
        tout = it.fn(tin)
        if tout is not None and it.m == 0:
            kind = 'x' if it.pri == 2.5 else 'v'
            prev = [tk for (_, tk, k) in toks if k == kind]
            if prev:
                tout = tout | prev[-1]
            toks.append((tv + it.v / VR, tout, kind))
        t0 = tv
        tv += it.v / VR
        end = tv
        if it.m > 0:
            tm = max(tm, t0) + it.m
            end = max(tm, tv) if it.lat else tv
        s['ready'] = end + it.lat


def _kernel(z_ref, q_hbm, k_hbm, v_hbm, sk_hbm, h_hbm, dd_hbm, wqkv_hbm, wo_hbm, f_hbm, g_hbm,
            o_hbm,
            sk_ref, dd_ref, f_ref, g_ref,
            qb, kb, vb, hb, wqkv, wo, wqp, wktp, KF, KV,
            U0, U1, U2, U3, H0, H1, H2, H3, RA, ZS, Y, X1, X3, Q1, Q2,
            XNa, XNb, PKa, PKb, PNa, PNb, PNc, PNd, Oa, Ob, P, ZP, Mp, Zm, ob, sems, osems, sem0):

    def cp_k(g): return pltpu.make_async_copy(k_hbm.at[pl.ds(g * SB, SB)], kb.at[pl.ds(HALO + g * SB, SB)], sems.at[g - 1])
    def cp_v(g): return pltpu.make_async_copy(v_hbm.at[pl.ds(g * SB, SB)], vb.at[pl.ds(g * SB, SB)], sems.at[2 + g])
    def cp_h(g): return pltpu.make_async_copy(h_hbm.at[:, pl.ds(g * SB, SB)], hb.at[:, pl.ds(g * SB, SB)], sems.at[5 + g])
    def cp_q(g): return pltpu.make_async_copy(q_hbm.at[pl.ds(g * SB, SB)], qb.at[pl.ds(g * SB, SB)], sems.at[9 + g])
    cp_w = pltpu.make_async_copy(wqkv_hbm.at[:, pl.ds(0, 2 * D)], wqkv.at[:, pl.ds(0, 2 * D)], sems.at[13])
    cp_wv = pltpu.make_async_copy(wqkv_hbm.at[:, pl.ds(2 * D, D)], wqkv.at[:, pl.ds(2 * D, D)], sems.at[14])
    cp_o = pltpu.make_async_copy(wo_hbm, wo, sems.at[15])

    cp_small = [pltpu.make_async_copy(a, b, sems.at[16 + i])
                for i, (a, b) in enumerate(((f_hbm, f_ref), (sk_hbm, sk_ref), (dd_hbm, dd_ref), (g_hbm, g_ref)))]

    def cp_sb(g):
        return cp_h(g), cp_k(g), cp_v(g)

    def cp0(j):
        cs = pl.ds(_mo(j * 128, 128), 128)
        return (pltpu.make_async_copy(h_hbm.at[cs, pl.ds(0, SB)], hb.at[cs, pl.ds(0, SB)], sem0.at[0, j]),
                pltpu.make_async_copy(k_hbm.at[pl.ds(0, SB), cs], kb.at[pl.ds(HALO, SB), cs], sem0.at[1, j]),
                pltpu.make_async_copy(v_hbm.at[pl.ds(0, SB), cs], vb.at[pl.ds(0, SB), cs], sem0.at[2, j]))

    def ocp(i):
        r0 = pl.multiple_of(i * T, T)
        return pltpu.make_async_copy(ob.at[pl.ds(r0, T)], o_hbm.at[pl.ds(r0, T)], osems.at[i])

    def start(*cs):
        for c in cs:
            c.start()

    def wait(*cs):
        for c in cs:
            c.wait()

    start(*cp0(0))
    start(*cp_small)
    for j in range(1, NT):
        start(*cp0(j))
    start(*cp_sb(1))

    kb[pl.ds(0, HALO), :] = jnp.zeros((HALO, D), BF16)
    P[...] = jnp.zeros(P.shape, F32)
    ZP[...] = jnp.zeros(ZP.shape, F32)
    XNa[...] = jnp.zeros(XNa.shape, U32)

    h2 = T // 2
    zi = z_ref[0]
    zm = jnp.full((8, 128), zi, jnp.int32).astype(U32)

    def tokof(u):
        return u[-8:, -128:] & zm

    def tokst(r):
        u = pltpu.bitcast(jnp.broadcast_to(r, (r.shape[0], 128)), U32)
        t = u[0:8]
        for k in range(1, r.shape[0] // 8):
            t = t | u[8 * k:8 * k + 8]
        return t & zm

    XN = (XNa, XNb); PK = (PKa, PKb); PN = (PNa, PNb, PNc, PNd); OO = (Oa, Ob)
    UC = (U0, U1, U2, U3); HC = (H0, H1, H2, H3)

    def pre_items(g, j):
        cs = pl.ds(_mo(j * 128, 128), 128)

        def dtile():
            dd = dd_ref[...].astype(F32)
            row = lax.broadcasted_iota(jnp.int32, (NT, 128), 0)
            return jnp.sum(jnp.where(row == j, dd, 0.0), axis=0, keepdims=True)

        def spec_store(dst, i, val, e, is_h):
            for gi in range(8):
                re = val[16 * gi:16 * gi + 8]
                im = val[16 * gi + 8:16 * gi + 16]
                rs = pl.ds(e * h2 + 8 * gi, 8)
                if is_h:
                    if g == 0 and i == 0:
                        re = re + dtile()
                    dst[j, i, 0, rs, :] = re + im
                    dst[j, i, 1, rs, :] = re
                    dst[j, i, 2, rs, :] = im
                else:
                    dst[j, i, 0, rs, :] = re
                    dst[j, i, 1, rs, :] = im - re
                    dst[j, i, 2, rs, :] = re + im

        def a_dot(i, e):
            def fn(tok):
                a_ = _nt(_bf(_gate(f_ref[e * 64:(e + 1) * 64, :], tok)), hb[cs, pl.ds((4 * g + i) * T, T)])
                spec_store(HC[g], i, a_, e, True)
            return Item(32, 20, 0, fn, 3)

        def kf(i):
            def fn(tok):
                n = T + (HALO if i == 0 else 0)
                o = 0 if i == 0 else HALO + i * T
                KF[0, o:o + n, :] = kb[pl.ds(g * SB + o, n), cs].astype(F32)
            return Item(0, 20, 0, fn, 3)

        def shift(i, hf):
            def fn(tok):
                sk = sk_ref[:, cs].astype(F32)
                o = HALO + i * T + hf * h2
                ks = KF[zi, o:o + h2, :] * sk[0:1]
                for s in range(1, 4):
                    ks = ks + KF[zi, o - s:o - s + h2, :] * sk[s:s + 1]
                kv = _pk(ks * vb[pl.ds((4 * g + i) * T + hf * h2, h2), cs].astype(F32))
                KV[i, hf * 32:(hf + 1) * 32, :] = kv
                return tokof(kv)
            return Item(0, 80, 0, fn, 3)

        def u_dot(i, e):
            def fn(tok):
                u = _nn(_bf(_gate(f_ref[e * 64:(e + 1) * 64, :], tok)), _bf(KV[i + zi]))
                spec_store(UC[g], i, u, e, False)
            return Item(32, 16, 0, fn, 3)

        items = [a_dot(0, 0), a_dot(0, 1)]
        for i in range(4):
            items += [kf(i), shift(i, 0), shift(i, 1)]
            if i < 3:
                items += [a_dot(i + 1, 0), a_dot(i + 1, 1)]
            items += [u_dot(i, 0), u_dot(i, 1)]
        return items

    def mac_items(g, j):
        def mac(fi):
            fs = pl.ds(fi * 8, 8)

            def fn(tok):
                acc = [[None] * 3 for _ in range(4)]
                for l in range(4 * g + 4):
                    h = [HC[l // 4][j, l % 4, c, fs, :] for c in range(3)]
                    for o in range(4):
                        m = 4 * g + o - l
                        if m < 0:
                            continue
                        for c in range(3):
                            t = h[c] * UC[m // 4][j, m % 4, c, fs, :]
                            acc[o][c] = t if acc[o][c] is None else acc[o][c] + t
                yr = [acc[o][0] - acc[o][2] for o in range(4)]
                yi = [acc[o][0] + acc[o][1] for o in range(4)]
                allz = None
                for o in range(4):
                    if o == 0 and g == 0:
                        zr, zi_ = yr[0], yi[0]
                    else:
                        pr, pi = (RA[j, 0, fs, :], RA[j, 1, fs, :]) if o == 0 else (yr[o - 1], yi[o - 1])
                        if fi < 8:
                            zr, zi_ = yr[o] - pi, yi[o] + pr
                        else:
                            zr, zi_ = yr[o] + pi, yi[o] - pr
                    zp_ = _pk(jnp.concatenate([zr, zi_], axis=0))
                    ZS[j, fs, o * 128:(o + 1) * 128] = zp_
                    allz = zp_ if allz is None else allz | zp_
                if g < NG - 1:
                    RA[j, 0, fs, :] = yr[3]
                    RA[j, 1, fs, :] = yi[3]
                return tokof(allz)
            return Item(0, 6 * (16 * g + 10) + 20, 0, fn, 1)
        return [mac(fi) for fi in range(T // 8)]

    def inv_items(g, j):
        cs = pl.ds(_mo(j * 128, 128), 128)

        def inv(i):
            def fn(tok):
                Y[pl.ds((4 * g + i) * T, T), cs] = _nn(_bf(_gate(g_ref[...], tok)),
                                                       _bf(ZS[j + zi, :, i * 128:(i + 1) * 128]))
            return Item(64, 16, 0, fn, 3)
        return [inv(i) for i in range(4)]

    def proj_items(r, Qo, par):
        xn, pkt = XN[par], PK[par]
        r0h = _mo(r * 64, 64)

        def kdot(n):
            def fn(tok):
                pk = _phi(_nt(_bf(_gate(wktp[n * 64:(n + 1) * 64, :], tok)), _bf(xn[zi])))
                ZP[n * 128:(n + 1) * 128, :] += pk
                pkt[0, n * 64:(n + 1) * 64, :] = _pk(pk)
            return Item(128, 160, 0, fn)

        def qdot(n):
            def fn(tok):
                ns = slice(n * 128, (n + 1) * 128)
                Qo[pl.ds(r0h, 64), ns] = _pk(_nn(_bf(_gate(xn[zi], tok)), _bf(wqp[:, ns])))
            return Item(128, 56, 0, fn)

        def pdot(n):
            def fn(tok):
                P[n * 128:(n + 1) * 128, :] += _nn(_bf(_gate(pkt[zi, n * 64:(n + 1) * 64, :], tok)), _bf(xn[zi]))
            return Item(128, 64, 0, fn)
        return [f(n) for f in (kdot, qdot, pdot) for n in range(4)]

    def ln_items(r, get_x, Xo, par):
        nc = T // RC
        st = {}

        def rows(c):
            return pl.ds(_mo(r * T + c * RC, RC), RC)

        def rowsz(c):
            return pl.ds(pl.multiple_of(r * T + (c + zi) * RC, RC), RC)

        def sa(c):
            def fn(tok):
                st['a', c] = _stats(get_x(c, rows(c)))
                return tokst(st['a', c][1])
            return Item(0, 90, LAT_X if c == nc - 1 else 0, fn, 2.5)

        def sb(c):
            def fn(tok):
                m, rs_ = st['a', c]
                x = get_x(c, rows(c))
                x1 = x + (x - m) * rs_ * Y[rows(c), :]
                Xo[rows(c), :] = x1
                st['b', c] = _stats(x1)
                return tokst(st['b', c][1])
            return Item(0, 150, LAT_X if c == nc - 1 else 0, fn, 2.5)

        def sc(c):
            def fn(tok):
                m, rs_ = st['b', c]
                xn = _pk((Xo[rowsz(c), :] - m) * rs_)
                XN[par][0, c * RC // 2:(c + 1) * RC // 2, :] = xn
                return tokof(xn)
            return Item(0, 45, 0, fn, 2.5)
        return [f(c) for f in (sa, sb) for c in range(nc)], [sc(c) for c in range(nc)]

    def d1_streams(r):
        ab, c_ = ln_items(r, lambda c, rs: qb[rs, :].astype(F32), X1, 0)
        for it in c_:
            it.after = 1
        return [proj_items(jnp.maximum(r - 1, 0), Q1, 0) + c_, ab]

    def wprep_items(n):
        ns = pl.ds(_mo(n * 128, 128), 128)

        def f1(tok):
            wqp[:, ns] = pltpu.bitcast(wqkv[:, ns], U32)

        def f2(tok):
            wktp[pl.ds(_mo(n * 64, 64), 64), :] = pltpu.bitcast(wqkv[:, pl.ds(_mo(D + n * 128, 128), 128)].T, U32)
        return [Item(0, 40, 0, f1), Item(0, 200, 0, f2)]

    rr = lax.broadcasted_iota(jnp.int32, (128, 128), 0) // DH
    cc = lax.broadcasted_iota(jnp.int32, (128, 128), 1) // DH
    mask = rr == cc

    def finish_items():
        st = {}

        def fkv(g):
            def fn(tok):
                sl = slice(g * 128, (g + 1) * 128)
                kvg = _nn(P[sl, :].astype(BF16), wqkv[:, 2 * D + g * 128:2 * D + (g + 1) * 128])
                st[g] = jnp.where(mask, kvg, 0.0).astype(BF16)
                P[sl, :] = jnp.zeros((128, D), F32)
            return Item(128, 150, 0, fn)

        def fz(g):
            def fn(tok):
                sl = slice(g * 128, (g + 1) * 128)
                z = jnp.sum(ZP[sl, :], axis=-1, keepdims=True)
                Zm[g] = _pk(jnp.where(mask, jnp.broadcast_to(z, (128, 128)), 0.0))
                ZP[sl, :] = jnp.zeros((128, 128), F32)
            return Item(0, 60, 0, fn)

        def fm(g):
            def fn(tok):
                Mp[g * 64:(g + 1) * 64, :] = _pk(_nn(st[g], wo[g * 128:(g + 1) * 128, :]))
            return Item(128, 80, 0, fn)
        return [f(g) for f in (fkv, fz, fm) for g in range(4)]

    def attn_items(r, Qi, par, sink):
        r0h = _mo(r * 64, 64)
        pn = PN[par]

        def e1(g):
            def fn(tok):
                sl = slice(g * 128, (g + 1) * 128)
                pq = _phi(_bf(_gate(Qi[pl.ds(r0h, 64), sl], tok)).astype(F32))
                den = _nn(pq.astype(BF16), _bf(Zm[g])) + 1e-6
                pn[0, :, sl] = _pk(pq * pl.reciprocal(den, approx=True))
            return Item(32, 150, LAT_M if g == 3 else 0, fn, 3)

        def e3(n):
            def fn(tok):
                sink(n, _nn(_bf(_gate(pn[zi], tok)), _bf(Mp[:, n * 128:(n + 1) * 128])))
            return Item(128, 70, LAT_M if n == 3 else 0, fn, 3)
        return [e1(g) for g in range(4)] + [e3(n) for n in range(4)]

    def att2_items(r, par):
        def sink(n, val):
            ns = slice(n * 128, (n + 1) * 128)
            OO[par][0, :, ns] = val + X1[pl.ds(_mo(r * T, T), T), ns]
        return attn_items(r, Q1, par, sink)

    def ln2_items(r, par):
        ab, c_ = ln_items(r, lambda c, rs: OO[par][zi, c * RC:(c + 1) * RC, :], X3, par)
        return ab + c_

    def att3_items(r, par):
        r0 = _mo(r * T, T)

        def sink(n, val):
            ns = slice(n * 128, (n + 1) * 128)
            ob[pl.ds(r0, T), ns] = (val + X3[pl.ds(r0, T), ns]).astype(BF16)
        return attn_items(r, Q2, par, sink)

    wait(*cp_small)

    def bpre(j, _):
        wait(*cp0(j))
        _merge(pre_items(0, j))
        return 0
    lax.fori_loop(0, NT, bpre, 0)
    start(cp_w, cp_q(0), *cp_sb(2))

    for g in range(NG + 1):
        if g + 1 < NG:
            wait(*cp_sb(g + 1))
        if g >= 1:
            wait(cp_q(g - 1))
        if g == 1:
            start(cp_q(1), *cp_sb(3))
        if g == 2:
            start(cp_q(2), cp_q(3), cp_wv, cp_o)

        def bg(j, _, g=g):
            streams = []
            if g >= 1:
                streams += d1_streams(4 * (g - 1) + j)
            if g + 1 < NG:
                streams.append(pre_items(g + 1, j))
            if g < NG:
                streams.append(mac_items(g, j) + inv_items(g, j))
            _merge(*streams, paced=(0,) if g >= 1 else (), pace=1.1, pin=(1 <= g < NG))
            if g == 0:
                @pl.when(j == 2)
                def _():
                    wait(cp_w)

                @pl.when(j >= 2)
                def _():
                    _merge(wprep_items(2 * (j - 2)), wprep_items(2 * (j - 2) + 1))
            if g == 1:
                @pl.when(j == 0)
                def _():
                    ZP[...] = jnp.zeros(ZP.shape, F32)
            return 0
        lax.fori_loop(0, NT, bg, 0)
    wait(cp_wv, cp_o)
    _merge(proj_items(NB - 1, Q1, 0) + finish_items())

    _merge(att2_items(0, 0))
    _merge(ln2_items(0, 0), att2_items(1, 1))

    def ph2(i, _):
        a = 2 * i
        c = lambda x: jnp.minimum(x, NB - 1)
        _merge(proj_items(a, Q2, 0), ln2_items(a + 1, 1), att2_items(c(a + 2), 0), paced=(0,))
        _merge(proj_items(a + 1, Q2, 1), ln2_items(c(a + 2), 0), att2_items(c(a + 3), 1), paced=(0,))
        return 0
    lax.fori_loop(0, NB // 2, ph2, 0)
    _merge(finish_items())

    def e1s(r, par):
        return att3_items(r, par)[:4]

    def e3s(r, par):
        return att3_items(r, par)[4:]

    _merge(e1s(0, 0), e1s(1, 1))

    def ph3(i, _):
        a = 4 * i
        c = lambda x: jnp.minimum(x, NB - 1)
        _merge(e3s(a, 0), e3s(a + 1, 1), e1s(a + 2, 2), e1s(a + 3, 3))
        start(ocp(a), ocp(a + 1))
        _merge(e3s(a + 2, 2), e3s(a + 3, 3), e1s(c(a + 4), 0), e1s(c(a + 5), 1))
        start(ocp(a + 2), ocp(a + 3))
        return 0
    lax.fori_loop(0, NB // 4, ph3, 0)

    def wt(i, _):
        ocp(i).wait()
        return 0
    lax.fori_loop(0, NB, wt, 0)


@jax.jit
def pallas_interleave_layers__ssm_conv_h3__linear_attn_block__prompt_kernel(
    A_q: jax.Array,
    A_k: jax.Array,
    A_v: jax.Array,
    A_shift_k: jax.Array,
    A_ssm_k: jax.Array,
    A_ssm_D: jax.Array,
    B_x: jax.Array,
    B_wqkv: jax.Array,
    B_wo: jax.Array,
):
    fwd, inv = _dft_mats()
    anyspec = pl.BlockSpec(memory_space=pl.ANY)
    half = lambda r, c: pltpu.VMEM((r // 2, c), U32)
    half1 = lambda r, c: pltpu.VMEM((1, r // 2, c), U32)
    spec = pltpu.VMEM((NT, 4, 3, T, 128), F32)
    out = pl.pallas_call(
        _kernel,
        out_shape=jax.ShapeDtypeStruct((S, D), BF16),
        in_specs=[pl.BlockSpec(memory_space=pltpu.SMEM)] + [anyspec] * 10,
        out_specs=anyspec,
        scratch_shapes=[
            pltpu.VMEM((4, D), BF16),
            pltpu.VMEM((NT, 128), BF16),
            half(2 * T, T), half(T, 2 * T),
            pltpu.VMEM((S, D), BF16),
            pltpu.VMEM((S + HALO, D), BF16),
            pltpu.VMEM((S, D), BF16),
            pltpu.VMEM((D, S), BF16),
            pltpu.VMEM((D, 3 * D), BF16),
            pltpu.VMEM((D, D), BF16),
            half(D, D),
            half(D, D),
            pltpu.VMEM((1, SB + HALO, 128), F32),
            pltpu.VMEM((4, T // 2, 128), U32),
            spec, spec, spec, spec,
            spec, spec, spec, spec,
            pltpu.VMEM((NT, 2, T, 128), F32),
            pltpu.VMEM((NT, T, D), U32),
            pltpu.VMEM((S, D), F32),
            pltpu.VMEM((S, D), F32),
            pltpu.VMEM((S, D), F32),
            half(S, D), half(S, D),
            half1(T, D), half1(T, D),
            half1(D, T), half1(D, T),
            half1(T, D), half1(T, D), half1(T, D), half1(T, D),
            pltpu.VMEM((1, T, D), F32), pltpu.VMEM((1, T, D), F32),
            pltpu.VMEM((D, D), F32),
            pltpu.VMEM((D, 128), F32),
            half(D, D),
            pltpu.VMEM((4, 64, 128), U32),
            pltpu.VMEM((S, D), BF16),
            pltpu.SemaphoreType.DMA((20,)),
            pltpu.SemaphoreType.DMA((NB,)),
            pltpu.SemaphoreType.DMA((3, NT)),
        ],
        compiler_params=pltpu.CompilerParams(vmem_limit_bytes=110 * 1024 * 1024),
    )(jnp.zeros((1,), jnp.int32), A_q.reshape(S, D), A_k.reshape(S, D), A_v.reshape(S, D), A_shift_k.T, A_ssm_k,
      A_ssm_D.reshape(NT, 128), B_wqkv, B_wo, jnp.asarray(fwd), jnp.asarray(inv))
    return out.reshape(1, S, D)
```

```python
import numpy as np
import jax
import jax.numpy as jnp
from jax import lax
import jax.experimental.pallas as pl
import jax.experimental.pallas.tpu as pltpu

S, D = 2048, 512
T = 128
NB = S // T
NG = 4
SB = S // NG
NT = D // 128
DH = 16
HALO = 16
EPS_LN = 1e-5
RC = 16

LAT_M, LAT_X = 300.0, 80.0
VR = 4.0
SLACK_M, HUNGRY = 256.0, 32.0
LAGM, LAGX = 0.0, 200.0

F32 = jnp.float32
BF16 = jnp.bfloat16
U32 = jnp.uint32


def _pack_rows_np(a):
    u = np.ascontiguousarray(a, np.float32).view(np.uint32)
    b = ((u + 0x7FFF + ((u >> 16) & 1)) >> 16).astype(np.uint32)
    return (b[0::2] | (b[1::2] << 16)).astype(np.uint32)


def _dft_mats():
    n2 = 2 * T
    ks = np.concatenate([np.arange(0, T, 2), np.arange(1, T, 2)])
    th = np.pi * np.outer(2 * ks + 1, np.arange(T)) / n2
    c_, s_ = np.cos(th), -np.sin(th)
    fwd = np.stack([c_.reshape(T // 8, 8, T), s_.reshape(T // 8, 8, T)], 1).reshape(2 * T, T)
    inv = np.stack([c_.T.reshape(T, T // 8, 8), s_.T.reshape(T, T // 8, 8)], 2).reshape(T, 2 * T) * (2.0 / n2)
    return _pack_rows_np(fwd), _pack_rows_np(inv)


def _bf(u):
    return pltpu.bitcast(u, BF16)


def _pk(x):
    return pltpu.bitcast(x.astype(BF16), U32)


def _stats(x):
    m = jnp.sum(x, axis=-1, keepdims=True) * (1.0 / D)
    e2 = jnp.sum(x * x, axis=-1, keepdims=True) * (1.0 / D)
    return m, lax.rsqrt(jnp.maximum(e2 - m * m, 0.0) + EPS_LN)


def _phi(t):
    return jnp.where(t > 0, t + (1.0 + 1e-6), jnp.exp(t) + 1e-6)


def _nt(a, b):
    return lax.dot_general(a, b, (((1,), (1,)), ((), ())), preferred_element_type=F32)


def _nn(a, b):
    return jnp.dot(a, b, preferred_element_type=F32)


def _mo(x, n):
    return x if isinstance(x, int) else pl.multiple_of(x, n)


def _gate(u, tok):
    if tok is None:
        return u
    r, c = u.shape
    top = u[0:8, 0:128] | tok
    if c > 128:
        top = jnp.concatenate([top, u[0:8, 128:]], axis=1)
    if r > 8:
        top = jnp.concatenate([top, u[8:]], axis=0)
    return top


class Item:
    __slots__ = ('m', 'v', 'lat', 'fn', 'pri', 'after')

    def __init__(self, m, v, lat, fn, pri=2, after=None):
        self.m, self.v, self.lat, self.fn, self.pri, self.after = m, v, lat, fn, pri, after


def _merge(*streams, paced=(), pace=0.8, pin=False):
    st = [dict(items=list(s_), i=0, ready=0.0) for s_ in streams]
    tot_m = sum(it.m for s in st for it in s['items'])
    tot_v = sum(it.v for s in st for it in s['items']) / VR
    chain = max(sum(max(it.m, it.v / VR) + it.lat for it in s['items']) for s in st)
    horizon = max(tot_m, tot_v, chain) * pace
    tm = tv = 0.0
    toks = []
    head = lambda s: s['items'][s['i']]
    while True:
        live = [s for s in st if s['i'] < len(s['items'])]
        if not live:
            break
        free = [s for s in live if head(s).after is None or st[head(s).after]['i'] >= len(st[head(s).after]['items'])]

        def earliest(s):
            t = s['ready']
            if head(s).m > 0:
                t = max(t, tm - SLACK_M)
            if st.index(s) in paced:
                t = max(t, horizon * s['i'] / len(s['items']))
            return t
        ok = [s for s in free if earliest(s) <= tv]
        if ok:
            hungry = tm <= tv + HUNGRY
            s = max(ok, key=lambda s: ((head(s).m > 0) if hungry else 0, head(s).pri))
        else:
            s = min(free, key=earliest)
            tv = max(tv, min(earliest(s), max(s['ready'], tm - SLACK_M)))
        it = head(s)
        s['i'] += 1
        tin = None
        if it.m > 0 and pin:
            now = max(tv, tm)
            both = ([tk for (td, tk, k) in toks if k == 'v' and td + LAGM <= now][-1:]
                    + [tk for (td, tk, k) in toks if k == 'x' and td + LAGX <= now][-1:])
            tin = None if not both else (both[0] if len(both) == 1 else both[0] | both[1])
        tout = it.fn(tin)
        if tout is not None and it.m == 0:
            kind = 'x' if it.pri == 2.5 else 'v'
            prev = [tk for (_, tk, k) in toks if k == kind]
            if prev:
                tout = tout | prev[-1]
            toks.append((tv + it.v / VR, tout, kind))
        t0 = tv
        tv += it.v / VR
        end = tv
        if it.m > 0:
            tm = max(tm, t0) + it.m
            end = max(tm, tv) if it.lat else tv
        s['ready'] = end + it.lat


def _kernel(z_ref, q_hbm, k_hbm, v_hbm, sk_hbm, h_hbm, dd_hbm, wqkv_hbm, wo_hbm, f_hbm, g_hbm,
            o_hbm,
            sk_ref, dd_ref, f_ref, g_ref,
            qb, kb, vb, hb, wqkv, wo, wqp, wktp, KF, KV,
            U0, U1, U2, U3, H0, H1, H2, H3, RA, ZS, Y, X1, X3, Q1, Q2,
            XNa, XNb, PKa, PKb, PNa, PNb, PNc, PNd, Oa, Ob, P, ZP, Mp, Zm, ob, sems, osems, sem0):

    def cp_k(g): return pltpu.make_async_copy(k_hbm.at[pl.ds(g * SB, SB)], kb.at[pl.ds(HALO + g * SB, SB)], sems.at[g - 1])
    def cp_v(g): return pltpu.make_async_copy(v_hbm.at[pl.ds(g * SB, SB)], vb.at[pl.ds(g * SB, SB)], sems.at[2 + g])
    def cp_h(g): return pltpu.make_async_copy(h_hbm.at[:, pl.ds(g * SB, SB)], hb.at[:, pl.ds(g * SB, SB)], sems.at[5 + g])
    def cp_q(g): return pltpu.make_async_copy(q_hbm.at[pl.ds(g * SB, SB)], qb.at[pl.ds(g * SB, SB)], sems.at[9 + g])
    cp_w = pltpu.make_async_copy(wqkv_hbm.at[:, pl.ds(0, 2 * D)], wqkv.at[:, pl.ds(0, 2 * D)], sems.at[13])
    cp_wv = pltpu.make_async_copy(wqkv_hbm.at[:, pl.ds(2 * D, D)], wqkv.at[:, pl.ds(2 * D, D)], sems.at[14])
    cp_o = pltpu.make_async_copy(wo_hbm, wo, sems.at[15])

    cp_small = [pltpu.make_async_copy(a, b, sems.at[16 + i])
                for i, (a, b) in enumerate(((f_hbm, f_ref), (sk_hbm, sk_ref), (dd_hbm, dd_ref), (g_hbm, g_ref)))]

    def cp_sb(g):
        return cp_h(g), cp_k(g), cp_v(g)

    def cp0(j):
        cs = pl.ds(_mo(j * 128, 128), 128)
        return (pltpu.make_async_copy(h_hbm.at[cs, pl.ds(0, SB)], hb.at[cs, pl.ds(0, SB)], sem0.at[0, j]),
                pltpu.make_async_copy(k_hbm.at[pl.ds(0, SB), cs], kb.at[pl.ds(HALO, SB), cs], sem0.at[1, j]),
                pltpu.make_async_copy(v_hbm.at[pl.ds(0, SB), cs], vb.at[pl.ds(0, SB), cs], sem0.at[2, j]))

    def ocp(i):
        r0 = pl.multiple_of(i * T, T)
        return pltpu.make_async_copy(ob.at[pl.ds(r0, T)], o_hbm.at[pl.ds(r0, T)], osems.at[i])

    def start(*cs):
        for c in cs:
            c.start()

    def wait(*cs):
        for c in cs:
            c.wait()

    start(*cp0(0))
    start(*cp_small)
    for j in range(1, NT):
        start(*cp0(j))
    start(*cp_sb(1))

    kb[pl.ds(0, HALO), :] = jnp.zeros((HALO, D), BF16)
    P[...] = jnp.zeros(P.shape, F32)
    ZP[...] = jnp.zeros(ZP.shape, F32)
    XNa[...] = jnp.zeros(XNa.shape, U32)

    h2 = T // 2
    zi = z_ref[0]
    zm = jnp.full((8, 128), zi, jnp.int32).astype(U32)

    def tokof(u):
        return u[-8:, -128:] & zm

    def tokst(r):
        u = pltpu.bitcast(jnp.broadcast_to(r, (r.shape[0], 128)), U32)
        t = u[0:8]
        for k in range(1, r.shape[0] // 8):
            t = t | u[8 * k:8 * k + 8]
        return t & zm

    XN = (XNa, XNb); PK = (PKa, PKb); PN = (PNa, PNb, PNc, PNd); OO = (Oa, Ob)
    UC = (U0, U1, U2, U3); HC = (H0, H1, H2, H3)

    def pre_items(g, j):
        cs = pl.ds(_mo(j * 128, 128), 128)

        def dtile():
            dd = dd_ref[...].astype(F32)
            row = lax.broadcasted_iota(jnp.int32, (NT, 128), 0)
            return jnp.sum(jnp.where(row == j, dd, 0.0), axis=0, keepdims=True)

        def spec_store(dst, i, val, e, is_h):
            for gi in range(8):
                re = val[16 * gi:16 * gi + 8]
                im = val[16 * gi + 8:16 * gi + 16]
                rs = pl.ds(e * h2 + 8 * gi, 8)
                if is_h:
                    if g == 0 and i == 0:
                        re = re + dtile()
                    dst[j, i, 0, rs, :] = re + im
                    dst[j, i, 1, rs, :] = re
                    dst[j, i, 2, rs, :] = im
                else:
                    dst[j, i, 0, rs, :] = re
                    dst[j, i, 1, rs, :] = im - re
                    dst[j, i, 2, rs, :] = re + im

        def a_dot(i, e):
            def fn(tok):
                a_ = _nt(_bf(_gate(f_ref[e * 64:(e + 1) * 64, :], tok)), hb[cs, pl.ds((4 * g + i) * T, T)])
                spec_store(HC[g], i, a_, e, True)
            return Item(32, 20, 0, fn, 3)

        def kf(i):
            def fn(tok):
                n = T + (HALO if i == 0 else 0)
                o = 0 if i == 0 else HALO + i * T
                KF[0, o:o + n, :] = kb[pl.ds(g * SB + o, n), cs].astype(F32)
            return Item(0, 20, 0, fn, 3)

        def shift(i, hf):
            def fn(tok):
                sk = sk_ref[:, cs].astype(F32)
                o = HALO + i * T + hf * h2
                ks = KF[zi, o:o + h2, :] * sk[0:1]
                for s in range(1, 4):
                    ks = ks + KF[zi, o - s:o - s + h2, :] * sk[s:s + 1]
                kv = _pk(ks * vb[pl.ds((4 * g + i) * T + hf * h2, h2), cs].astype(F32))
                KV[i, hf * 32:(hf + 1) * 32, :] = kv
                return tokof(kv)
            return Item(0, 80, 0, fn, 3)

        def u_dot(i, e):
            def fn(tok):
                u = _nn(_bf(_gate(f_ref[e * 64:(e + 1) * 64, :], tok)), _bf(KV[i + zi]))
                spec_store(UC[g], i, u, e, False)
            return Item(32, 16, 0, fn, 3)

        items = [a_dot(0, 0), a_dot(0, 1)]
        for i in range(4):
            items += [kf(i), shift(i, 0), shift(i, 1)]
            if i < 3:
                items += [a_dot(i + 1, 0), a_dot(i + 1, 1)]
            items += [u_dot(i, 0), u_dot(i, 1)]
        return items

    def mac_items(g, j):
        def mac(fi):
            fs = pl.ds(fi * 8, 8)

            def fn(tok):
                acc = [[None] * 3 for _ in range(4)]
                for l in range(4 * g + 4):
                    h = [HC[l // 4][j, l % 4, c, fs, :] for c in range(3)]
                    for o in range(4):
                        m = 4 * g + o - l
                        if m < 0:
                            continue
                        for c in range(3):
                            t = h[c] * UC[m // 4][j, m % 4, c, fs, :]
                            acc[o][c] = t if acc[o][c] is None else acc[o][c] + t
                yr = [acc[o][0] - acc[o][2] for o in range(4)]
                yi = [acc[o][0] + acc[o][1] for o in range(4)]
                allz = None
                for o in range(4):
                    if o == 0 and g == 0:
                        zr, zi_ = yr[0], yi[0]
                    else:
                        pr, pi = (RA[j, 0, fs, :], RA[j, 1, fs, :]) if o == 0 else (yr[o - 1], yi[o - 1])
                        if fi < 8:
                            zr, zi_ = yr[o] - pi, yi[o] + pr
                        else:
                            zr, zi_ = yr[o] + pi, yi[o] - pr
                    zp_ = _pk(jnp.concatenate([zr, zi_], axis=0))
                    ZS[j, fs, o * 128:(o + 1) * 128] = zp_
                    allz = zp_ if allz is None else allz | zp_
                if g < NG - 1:
                    RA[j, 0, fs, :] = yr[3]
                    RA[j, 1, fs, :] = yi[3]
                return tokof(allz)
            return Item(0, 6 * (16 * g + 10) + 20, 0, fn, 1)
        return [mac(fi) for fi in range(T // 8)]

    def inv_items(g, j):
        cs = pl.ds(_mo(j * 128, 128), 128)

        def inv(i):
            def fn(tok):
                Y[pl.ds((4 * g + i) * T, T), cs] = _nn(_bf(_gate(g_ref[...], tok)),
                                                       _bf(ZS[j + zi, :, i * 128:(i + 1) * 128]))
            return Item(64, 16, 0, fn, 3)
        return [inv(i) for i in range(4)]

    def proj_items(r, Qo, par):
        xn, pkt = XN[par], PK[par]
        r0h = _mo(r * 64, 64)

        def kdot(n):
            def fn(tok):
                pk = _phi(_nt(_bf(_gate(wktp[n * 64:(n + 1) * 64, :], tok)), _bf(xn[zi])))
                ZP[n * 128:(n + 1) * 128, :] += pk
                pkt[0, n * 64:(n + 1) * 64, :] = _pk(pk)
            return Item(128, 160, 0, fn)

        def qdot(n):
            def fn(tok):
                ns = slice(n * 128, (n + 1) * 128)
                Qo[pl.ds(r0h, 64), ns] = _pk(_nn(_bf(_gate(xn[zi], tok)), _bf(wqp[:, ns])))
            return Item(128, 56, 0, fn)

        def pdot(n):
            def fn(tok):
                P[n * 128:(n + 1) * 128, :] += _nn(_bf(_gate(pkt[zi, n * 64:(n + 1) * 64, :], tok)), _bf(xn[zi]))
            return Item(128, 64, 0, fn)
        return [f(n) for f in (kdot, qdot, pdot) for n in range(4)]

    def ln_items(r, get_x, Xo, par):
        nc = T // RC
        st = {}

        def rows(c):
            return pl.ds(_mo(r * T + c * RC, RC), RC)

        def rowsz(c):
            return pl.ds(pl.multiple_of(r * T + (c + zi) * RC, RC), RC)

        def sa(c):
            def fn(tok):
                st['a', c] = _stats(get_x(c, rows(c)))
                return tokst(st['a', c][1])
            return Item(0, 45, LAT_X if c == nc - 1 else 0, fn, 2.5)

        def sb(c):
            def fn(tok):
                m, rs_ = st['a', c]
                x = get_x(c, rows(c))
                x1 = x + (x - m) * rs_ * Y[rows(c), :]
                Xo[rows(c), :] = x1
                st['b', c] = _stats(x1)
                return tokst(st['b', c][1])
            return Item(0, 75, LAT_X if c == nc - 1 else 0, fn, 2.5)

        def sc(c):
            def fn(tok):
                m, rs_ = st['b', c]
                xn = _pk((Xo[rowsz(c), :] - m) * rs_)
                XN[par][0, c * RC // 2:(c + 1) * RC // 2, :] = xn
                return tokof(xn)
            return Item(0, 22.5, 0, fn, 2.5)
        return [f(c) for f in (sa, sb) for c in range(nc)], [sc(c) for c in range(nc)]

    def d1_streams(r):
        ab, c_ = ln_items(r, lambda c, rs: qb[rs, :].astype(F32), X1, 0)
        for it in c_:
            it.after = 1
        return [proj_items(jnp.maximum(r - 1, 0), Q1, 0) + c_, ab]

    def wprep_items(n):
        ns = pl.ds(_mo(n * 128, 128), 128)

        def f1(tok):
            wqp[:, ns] = pltpu.bitcast(wqkv[:, ns], U32)

        def f2(tok):
            wktp[pl.ds(_mo(n * 64, 64), 64), :] = pltpu.bitcast(wqkv[:, pl.ds(_mo(D + n * 128, 128), 128)].T, U32)
        return [Item(0, 40, 0, f1), Item(0, 200, 0, f2)]

    rr = lax.broadcasted_iota(jnp.int32, (128, 128), 0) // DH
    cc = lax.broadcasted_iota(jnp.int32, (128, 128), 1) // DH
    mask = rr == cc

    def finish_items():
        st = {}

        def fkv(g):
            def fn(tok):
                sl = slice(g * 128, (g + 1) * 128)
                kvg = _nn(P[sl, :].astype(BF16), wqkv[:, 2 * D + g * 128:2 * D + (g + 1) * 128])
                st[g] = jnp.where(mask, kvg, 0.0).astype(BF16)
                P[sl, :] = jnp.zeros((128, D), F32)
            return Item(128, 150, 0, fn)

        def fz(g):
            def fn(tok):
                sl = slice(g * 128, (g + 1) * 128)
                z = jnp.sum(ZP[sl, :], axis=-1, keepdims=True)
                Zm[g] = _pk(jnp.where(mask, jnp.broadcast_to(z, (128, 128)), 0.0))
                ZP[sl, :] = jnp.zeros((128, 128), F32)
            return Item(0, 60, 0, fn)

        def fm(g):
            def fn(tok):
                Mp[g * 64:(g + 1) * 64, :] = _pk(_nn(st[g], wo[g * 128:(g + 1) * 128, :]))
            return Item(128, 80, 0, fn)
        return [f(g) for f in (fkv, fz, fm) for g in range(4)]

    def attn_items(r, Qi, par, sink):
        r0h = _mo(r * 64, 64)
        pn = PN[par]

        def e1(g):
            def fn(tok):
                sl = slice(g * 128, (g + 1) * 128)
                pq = _phi(_bf(_gate(Qi[pl.ds(r0h, 64), sl], tok)).astype(F32))
                den = _nn(pq.astype(BF16), _bf(Zm[g])) + 1e-6
                pn[0, :, sl] = _pk(pq * pl.reciprocal(den, approx=True))
            return Item(32, 150, LAT_M if g == 3 else 0, fn, 3)

        def e3(n):
            def fn(tok):
                sink(n, _nn(_bf(_gate(pn[zi], tok)), _bf(Mp[:, n * 128:(n + 1) * 128])))
            return Item(128, 70, LAT_M if n == 3 else 0, fn, 3)
        return [e1(g) for g in range(4)] + [e3(n) for n in range(4)]

    def att2_items(r, par):
        def sink(n, val):
            ns = slice(n * 128, (n + 1) * 128)
            OO[par][0, :, ns] = val + X1[pl.ds(_mo(r * T, T), T), ns]
        return attn_items(r, Q1, par, sink)

    def ln2_items(r, par):
        ab, c_ = ln_items(r, lambda c, rs: OO[par][zi, c * RC:(c + 1) * RC, :], X3, par)
        return ab + c_

    def att3_items(r, par):
        r0 = _mo(r * T, T)

        def sink(n, val):
            ns = slice(n * 128, (n + 1) * 128)
            ob[pl.ds(r0, T), ns] = (val + X3[pl.ds(r0, T), ns]).astype(BF16)
        return attn_items(r, Q2, par, sink)

    wait(*cp_small)

    def bpre(j, _):
        wait(*cp0(j))
        _merge(pre_items(0, j))
        return 0
    lax.fori_loop(0, NT, bpre, 0)
    start(cp_w, cp_q(0), *cp_sb(2))

    for g in range(NG + 1):
        if g + 1 < NG:
            wait(*cp_sb(g + 1))
        if g >= 1:
            wait(cp_q(g - 1))
        if g == 1:
            start(cp_q(1), *cp_sb(3))
        if g == 2:
            start(cp_q(2), cp_q(3), cp_wv, cp_o)

        def bg(j, _, g=g):
            streams = []
            if g >= 1:
                streams += d1_streams(4 * (g - 1) + j)
            if g + 1 < NG:
                streams.append(pre_items(g + 1, j))
            if g < NG:
                streams.append(mac_items(g, j) + inv_items(g, j))
            _merge(*streams, paced=(0,) if g >= 1 else (), pace=1.1, pin=(1 <= g < NG))
            if g == 0:
                @pl.when(j == 2)
                def _():
                    wait(cp_w)

                @pl.when(j >= 2)
                def _():
                    _merge(wprep_items(2 * (j - 2)), wprep_items(2 * (j - 2) + 1))
            if g == 1:
                @pl.when(j == 0)
                def _():
                    ZP[...] = jnp.zeros(ZP.shape, F32)
            return 0
        lax.fori_loop(0, NT, bg, 0)
    wait(cp_wv, cp_o)
    _merge(proj_items(NB - 1, Q1, 0) + finish_items())

    _merge(att2_items(0, 0))
    _merge(ln2_items(0, 0), att2_items(1, 1))

    def ph2(i, _):
        a = 2 * i
        c = lambda x: jnp.minimum(x, NB - 1)
        _merge(proj_items(a, Q2, 0), ln2_items(a + 1, 1), att2_items(c(a + 2), 0), paced=(0,))
        _merge(proj_items(a + 1, Q2, 1), ln2_items(c(a + 2), 0), att2_items(c(a + 3), 1), paced=(0,))
        return 0
    lax.fori_loop(0, NB // 2, ph2, 0)
    _merge(finish_items())

    def e1s(r, par):
        return att3_items(r, par)[:4]

    def e3s(r, par):
        return att3_items(r, par)[4:]

    _merge(e1s(0, 0), e1s(1, 1))

    def ph3(i, _):
        a = 4 * i
        c = lambda x: jnp.minimum(x, NB - 1)
        _merge(e3s(a, 0), e3s(a + 1, 1), e1s(a + 2, 2), e1s(a + 3, 3))
        start(ocp(a), ocp(a + 1))
        _merge(e3s(a + 2, 2), e3s(a + 3, 3), e1s(c(a + 4), 0), e1s(c(a + 5), 1))
        start(ocp(a + 2), ocp(a + 3))
        return 0
    lax.fori_loop(0, NB // 4, ph3, 0)

    def wt(i, _):
        ocp(i).wait()
        return 0
    lax.fori_loop(0, NB, wt, 0)


@jax.jit
def pallas_interleave_layers__ssm_conv_h3__linear_attn_block__prompt_kernel(
    A_q: jax.Array,
    A_k: jax.Array,
    A_v: jax.Array,
    A_shift_k: jax.Array,
    A_ssm_k: jax.Array,
    A_ssm_D: jax.Array,
    B_x: jax.Array,
    B_wqkv: jax.Array,
    B_wo: jax.Array,
):
    fwd, inv = _dft_mats()
    anyspec = pl.BlockSpec(memory_space=pl.ANY)
    half = lambda r, c: pltpu.VMEM((r // 2, c), U32)
    half1 = lambda r, c: pltpu.VMEM((1, r // 2, c), U32)
    spec = pltpu.VMEM((NT, 4, 3, T, 128), F32)
    out = pl.pallas_call(
        _kernel,
        out_shape=jax.ShapeDtypeStruct((S, D), BF16),
        in_specs=[pl.BlockSpec(memory_space=pltpu.SMEM)] + [anyspec] * 10,
        out_specs=anyspec,
        scratch_shapes=[
            pltpu.VMEM((4, D), BF16),
            pltpu.VMEM((NT, 128), BF16),
            half(2 * T, T), half(T, 2 * T),
            pltpu.VMEM((S, D), BF16),
            pltpu.VMEM((S + HALO, D), BF16),
            pltpu.VMEM((S, D), BF16),
            pltpu.VMEM((D, S), BF16),
            pltpu.VMEM((D, 3 * D), BF16),
            pltpu.VMEM((D, D), BF16),
            half(D, D),
            half(D, D),
            pltpu.VMEM((1, SB + HALO, 128), F32),
            pltpu.VMEM((4, T // 2, 128), U32),
            spec, spec, spec, spec,
            spec, spec, spec, spec,
            pltpu.VMEM((NT, 2, T, 128), F32),
            pltpu.VMEM((NT, T, D), U32),
            pltpu.VMEM((S, D), F32),
            pltpu.VMEM((S, D), F32),
            pltpu.VMEM((S, D), F32),
            half(S, D), half(S, D),
            half1(T, D), half1(T, D),
            half1(D, T), half1(D, T),
            half1(T, D), half1(T, D), half1(T, D), half1(T, D),
            pltpu.VMEM((1, T, D), F32), pltpu.VMEM((1, T, D), F32),
            pltpu.VMEM((D, D), F32),
            pltpu.VMEM((D, 128), F32),
            half(D, D),
            pltpu.VMEM((4, 64, 128), U32),
            pltpu.VMEM((S, D), BF16),
            pltpu.SemaphoreType.DMA((20,)),
            pltpu.SemaphoreType.DMA((NB,)),
            pltpu.SemaphoreType.DMA((3, NT)),
        ],
        compiler_params=pltpu.CompilerParams(vmem_limit_bytes=110 * 1024 * 1024),
    )(jnp.zeros((1,), jnp.int32), A_q.reshape(S, D), A_k.reshape(S, D), A_v.reshape(S, D), A_shift_k.T, A_ssm_k,
      A_ssm_D.reshape(NT, 128), B_wqkv, B_wo, jnp.asarray(fwd), jnp.asarray(inv))
    return out.reshape(1, S, D)
```

```python
import numpy as np
import jax
import jax.numpy as jnp
from jax import lax
import jax.experimental.pallas as pl
import jax.experimental.pallas.tpu as pltpu

S, D = 2048, 512
T = 128
NB = S // T
NG = 4
SB = S // NG
NT = D // 128
DH = 16
HALO = 16
EPS_LN = 1e-5
RC = 16

LAT_M, LAT_X = 300.0, 80.0
VR = 4.0
SLACK_M, HUNGRY = 256.0, 32.0
LAGM, LAGX = 0.0, 200.0

F32 = jnp.float32
BF16 = jnp.bfloat16
U32 = jnp.uint32


def _pack_rows_np(a):
    u = np.ascontiguousarray(a, np.float32).view(np.uint32)
    b = ((u + 0x7FFF + ((u >> 16) & 1)) >> 16).astype(np.uint32)
    return (b[0::2] | (b[1::2] << 16)).astype(np.uint32)


def _dft_mats():
    n2 = 2 * T
    ks = np.concatenate([np.arange(0, T, 2), np.arange(1, T, 2)])
    th = np.pi * np.outer(2 * ks + 1, np.arange(T)) / n2
    c_, s_ = np.cos(th), -np.sin(th)
    fwd = np.stack([c_.reshape(T // 8, 8, T), s_.reshape(T // 8, 8, T)], 1).reshape(2 * T, T)
    inv = np.stack([c_.T.reshape(T, T // 8, 8), s_.T.reshape(T, T // 8, 8)], 2).reshape(T, 2 * T) * (2.0 / n2)
    return _pack_rows_np(fwd), _pack_rows_np(inv)


def _bf(u):
    return pltpu.bitcast(u, BF16)


def _pk(x):
    return pltpu.bitcast(x.astype(BF16), U32)


def _stats(x):
    m = jnp.sum(x, axis=-1, keepdims=True) * (1.0 / D)
    e2 = jnp.sum(x * x, axis=-1, keepdims=True) * (1.0 / D)
    return m, lax.rsqrt(jnp.maximum(e2 - m * m, 0.0) + EPS_LN)


def _phi(t):
    return jnp.where(t > 0, t + (1.0 + 1e-6), jnp.exp(t) + 1e-6)


def _nt(a, b):
    return lax.dot_general(a, b, (((1,), (1,)), ((), ())), preferred_element_type=F32)


def _nn(a, b):
    return jnp.dot(a, b, preferred_element_type=F32)


def _mo(x, n):
    return x if isinstance(x, int) else pl.multiple_of(x, n)


def _gate(u, tok):
    if tok is None:
        return u
    r, c = u.shape
    top = u[0:8, 0:128] | tok
    if c > 128:
        top = jnp.concatenate([top, u[0:8, 128:]], axis=1)
    if r > 8:
        top = jnp.concatenate([top, u[8:]], axis=0)
    return top


class Item:
    __slots__ = ('m', 'v', 'lat', 'fn', 'pri', 'after')

    def __init__(self, m, v, lat, fn, pri=2, after=None):
        self.m, self.v, self.lat, self.fn, self.pri, self.after = m, v, lat, fn, pri, after


def _merge(*streams, paced=(), pace=0.8, pin=False):
    st = [dict(items=list(s_), i=0, ready=0.0) for s_ in streams]
    tot_m = sum(it.m for s in st for it in s['items'])
    tot_v = sum(it.v for s in st for it in s['items']) / VR
    chain = max(sum(max(it.m, it.v / VR) + it.lat for it in s['items']) for s in st)
    horizon = max(tot_m, tot_v, chain) * pace
    tm = tv = 0.0
    toks = []
    head = lambda s: s['items'][s['i']]
    while True:
        live = [s for s in st if s['i'] < len(s['items'])]
        if not live:
            break
        free = [s for s in live if head(s).after is None or st[head(s).after]['i'] >= len(st[head(s).after]['items'])]

        def earliest(s):
            t = s['ready']
            if head(s).m > 0:
                t = max(t, tm - SLACK_M)
            if st.index(s) in paced:
                t = max(t, horizon * s['i'] / len(s['items']))
            return t
        ok = [s for s in free if earliest(s) <= tv]
        if ok:
            hungry = tm <= tv + HUNGRY
            s = max(ok, key=lambda s: ((head(s).m > 0) if hungry else 0, head(s).pri))
        else:
            s = min(free, key=earliest)
            tv = max(tv, min(earliest(s), max(s['ready'], tm - SLACK_M)))
        it = head(s)
        s['i'] += 1
        tin = None
        if it.m > 0 and pin:
            now = max(tv, tm)
            both = ([tk for (td, tk, k) in toks if k == 'v' and td + LAGM <= now][-1:]
                    + [tk for (td, tk, k) in toks if k == 'x' and td + LAGX <= now][-1:])
            tin = None if not both else (both[0] if len(both) == 1 else both[0] | both[1])
        tout = it.fn(tin)
        if tout is not None and it.m == 0:
            kind = 'x' if it.pri == 2.5 else 'v'
            prev = [tk for (_, tk, k) in toks if k == kind]
            if prev:
                tout = tout | prev[-1]
            toks.append((tv + it.v / VR, tout, kind))
        t0 = tv
        tv += it.v / VR
        end = tv
        if it.m > 0:
            tm = max(tm, t0) + it.m
            end = max(tm, tv) if it.lat else tv
        s['ready'] = end + it.lat


def _kernel(z_ref, q_hbm, k_hbm, v_hbm, sk_hbm, h_hbm, dd_hbm, wqkv_hbm, wo_hbm, f_hbm, g_hbm,
            o_hbm,
            sk_ref, dd_ref, f_ref, g_ref,
            qb, kb, vb, hb, wqkv, wo, wqp, wktp, KF, KV,
            U0, U1, U2, U3, H0, H1, H2, H3, RA, ZS, Y, X1, X3, Q1, Q2,
            XNa, XNb, PKa, PKb, PNa, PNb, PNc, PNd, Oa, Ob, P, ZP, Mp, Zm, ob, sems, osems, sem0):

    def cp_k(g): return pltpu.make_async_copy(k_hbm.at[pl.ds(g * SB, SB)], kb.at[pl.ds(HALO + g * SB, SB)], sems.at[g - 1])
    def cp_v(g): return pltpu.make_async_copy(v_hbm.at[pl.ds(g * SB, SB)], vb.at[pl.ds(g * SB, SB)], sems.at[2 + g])
    def cp_h(g): return pltpu.make_async_copy(h_hbm.at[:, pl.ds(g * SB, SB)], hb.at[:, pl.ds(g * SB, SB)], sems.at[5 + g])
    def cp_q(g): return pltpu.make_async_copy(q_hbm.at[pl.ds(g * SB, SB)], qb.at[pl.ds(g * SB, SB)], sems.at[9 + g])
    cp_w = pltpu.make_async_copy(wqkv_hbm.at[:, pl.ds(0, 2 * D)], wqkv.at[:, pl.ds(0, 2 * D)], sems.at[13])
    cp_wv = pltpu.make_async_copy(wqkv_hbm.at[:, pl.ds(2 * D, D)], wqkv.at[:, pl.ds(2 * D, D)], sems.at[14])
    cp_o = pltpu.make_async_copy(wo_hbm, wo, sems.at[15])

    cp_small = [pltpu.make_async_copy(a, b, sems.at[16 + i])
                for i, (a, b) in enumerate(((f_hbm, f_ref), (sk_hbm, sk_ref), (dd_hbm, dd_ref), (g_hbm, g_ref)))]

    def cp_sb(g):
        return cp_h(g), cp_k(g), cp_v(g)

    def cp0(j):
        cs = pl.ds(_mo(j * 128, 128), 128)
        return (pltpu.make_async_copy(h_hbm.at[cs, pl.ds(0, SB)], hb.at[cs, pl.ds(0, SB)], sem0.at[j]),
                pltpu.make_async_copy(k_hbm.at[pl.ds(0, SB), cs], kb.at[pl.ds(HALO, SB), cs], sem0.at[NT + j]),
                pltpu.make_async_copy(v_hbm.at[pl.ds(0, SB), cs], vb.at[pl.ds(0, SB), cs], sem0.at[2 * NT + j]))

    def ocp(i):
        r0 = pl.multiple_of(i * T, T)
        return pltpu.make_async_copy(ob.at[pl.ds(r0, T)], o_hbm.at[pl.ds(r0, T)], osems.at[i])

    def start(*cs):
        for c in cs:
            c.start()

    def wait(*cs):
        for c in cs:
            c.wait()

    start(*cp0(0))
    start(*cp_small)
    for j in range(1, NT):
        start(*cp0(j))
    start(*cp_sb(1))

    kb[pl.ds(0, HALO), :] = jnp.zeros((HALO, D), BF16)
    P[...] = jnp.zeros(P.shape, F32)
    ZP[...] = jnp.zeros(ZP.shape, F32)
    XNa[...] = jnp.zeros(XNa.shape, U32)

    h2 = T // 2
    zi = z_ref[0]
    zm = jnp.full((8, 128), zi, jnp.int32).astype(U32)

    def tokof(u):
        return u[-8:, -128:] & zm

    def tokst(r):
        u = pltpu.bitcast(jnp.broadcast_to(r, (r.shape[0], 128)), U32)
        t = u[0:8]
        for k in range(1, r.shape[0] // 8):
            t = t | u[8 * k:8 * k + 8]
        return t & zm

    XN = (XNa, XNb); PK = (PKa, PKb); PN = (PNa, PNb, PNc, PNd); OO = (Oa, Ob)
    UC = (U0, U1, U2, U3); HC = (H0, H1, H2, H3)

    def pre_items(g, j):
        cs = pl.ds(_mo(j * 128, 128), 128)

        def dtile():
            dd = dd_ref[...].astype(F32)
            row = lax.broadcasted_iota(jnp.int32, (NT, 128), 0)
            return jnp.sum(jnp.where(row == j, dd, 0.0), axis=0, keepdims=True)

        def spec_store(dst, i, val, e, is_h):
            for gi in range(8):
                re = val[16 * gi:16 * gi + 8]
                im = val[16 * gi + 8:16 * gi + 16]
                rs = pl.ds(e * h2 + 8 * gi, 8)
                if is_h:
                    if g == 0 and i == 0:
                        re = re + dtile()
                    dst[j, i, 0, rs, :] = re + im
                    dst[j, i, 1, rs, :] = re
                    dst[j, i, 2, rs, :] = im
                else:
                    dst[j, i, 0, rs, :] = re
                    dst[j, i, 1, rs, :] = im - re
                    dst[j, i, 2, rs, :] = re + im

        def a_dot(i, e):
            def fn(tok):
                a_ = _nt(_bf(_gate(f_ref[e * 64:(e + 1) * 64, :], tok)), hb[cs, pl.ds((4 * g + i) * T, T)])
                spec_store(HC[g], i, a_, e, True)
            return Item(32, 20, 0, fn, 3)

        def kf(i):
            def fn(tok):
                n = T + (HALO if i == 0 else 0)
                o = 0 if i == 0 else HALO + i * T
                KF[0, o:o + n, :] = kb[pl.ds(g * SB + o, n), cs].astype(F32)
            return Item(0, 20, 0, fn, 3)

        def shift(i, hf):
            def fn(tok):
                sk = sk_ref[:, cs].astype(F32)
                o = HALO + i * T + hf * h2
                ks = KF[zi, o:o + h2, :] * sk[0:1]
                for s in range(1, 4):
                    ks = ks + KF[zi, o - s:o - s + h2, :] * sk[s:s + 1]
                kv = _pk(ks * vb[pl.ds((4 * g + i) * T + hf * h2, h2), cs].astype(F32))
                KV[i, hf * 32:(hf + 1) * 32, :] = kv
                return tokof(kv)
            return Item(0, 80, 0, fn, 3)

        def u_dot(i, e):
            def fn(tok):
                u = _nn(_bf(_gate(f_ref[e * 64:(e + 1) * 64, :], tok)), _bf(KV[i + zi]))
                spec_store(UC[g], i, u, e, False)
            return Item(32, 16, 0, fn, 3)

        items = [a_dot(0, 0), a_dot(0, 1)]
        for i in range(4):
            items += [kf(i), shift(i, 0), shift(i, 1)]
            if i < 3:
                items += [a_dot(i + 1, 0), a_dot(i + 1, 1)]
            items += [u_dot(i, 0), u_dot(i, 1)]
        return items

    def mac_items(g, j):
        def mac(fi):
            fs = pl.ds(fi * 8, 8)

            def fn(tok):
                acc = [[None] * 3 for _ in range(4)]
                for l in range(4 * g + 4):
                    h = [HC[l // 4][j, l % 4, c, fs, :] for c in range(3)]
                    for o in range(4):
                        m = 4 * g + o - l
                        if m < 0:
                            continue
                        for c in range(3):
                            t = h[c] * UC[m // 4][j, m % 4, c, fs, :]
                            acc[o][c] = t if acc[o][c] is None else acc[o][c] + t
                yr = [acc[o][0] - acc[o][2] for o in range(4)]
                yi = [acc[o][0] + acc[o][1] for o in range(4)]
                allz = None
                for o in range(4):
                    if o == 0 and g == 0:
                        zr, zi_ = yr[0], yi[0]
                    else:
                        pr, pi = (RA[j, 0, fs, :], RA[j, 1, fs, :]) if o == 0 else (yr[o - 1], yi[o - 1])
                        if fi < 8:
                            zr, zi_ = yr[o] - pi, yi[o] + pr
                        else:
                            zr, zi_ = yr[o] + pi, yi[o] - pr
                    zp_ = _pk(jnp.concatenate([zr, zi_], axis=0))
                    ZS[j, fs, o * 128:(o + 1) * 128] = zp_
                    allz = zp_ if allz is None else allz | zp_
                if g < NG - 1:
                    RA[j, 0, fs, :] = yr[3]
                    RA[j, 1, fs, :] = yi[3]
                return tokof(allz)
            return Item(0, 6 * (16 * g + 10) + 20, 0, fn, 1)
        return [mac(fi) for fi in range(T // 8)]

    def inv_items(g, j):
        cs = pl.ds(_mo(j * 128, 128), 128)

        def inv(i):
            def fn(tok):
                Y[pl.ds((4 * g + i) * T, T), cs] = _nn(_bf(_gate(g_ref[...], tok)),
                                                       _bf(ZS[j + zi, :, i * 128:(i + 1) * 128]))
            return Item(64, 16, 0, fn, 3)
        return [inv(i) for i in range(4)]

    def proj_items(r, Qo, par):
        xn, pkt = XN[par], PK[par]
        r0h = _mo(r * 64, 64)

        def kdot(n):
            def fn(tok):
                pk = _phi(_nt(_bf(_gate(wktp[n * 64:(n + 1) * 64, :], tok)), _bf(xn[zi])))
                ZP[n * 128:(n + 1) * 128, :] += pk
                pkt[0, n * 64:(n + 1) * 64, :] = _pk(pk)
            return Item(128, 160, 0, fn)

        def qdot(n):
            def fn(tok):
                ns = slice(n * 128, (n + 1) * 128)
                Qo[pl.ds(r0h, 64), ns] = _pk(_nn(_bf(_gate(xn[zi], tok)), _bf(wqp[:, ns])))
            return Item(128, 56, 0, fn)

        def pdot(n):
            def fn(tok):
                P[n * 128:(n + 1) * 128, :] += _nn(_bf(_gate(pkt[zi, n * 64:(n + 1) * 64, :], tok)), _bf(xn[zi]))
            return Item(128, 64, 0, fn)
        return [f(n) for f in (kdot, qdot, pdot) for n in range(4)]

    def ln_items(r, get_x, Xo, par):
        nc = T // RC
        st = {}

        def rows(c):
            return pl.ds(_mo(r * T + c * RC, RC), RC)

        def rowsz(c):
            return pl.ds(pl.multiple_of(r * T + (c + zi) * RC, RC), RC)

        def sa(c):
            def fn(tok):
                st['a', c] = _stats(get_x(c, rows(c)))
                return tokst(st['a', c][1])
            return Item(0, 45, LAT_X if c == nc - 1 else 0, fn, 2.5)

        def sb(c):
            def fn(tok):
                m, rs_ = st['a', c]
                x = get_x(c, rows(c))
                x1 = x + (x - m) * rs_ * Y[rows(c), :]
                Xo[rows(c), :] = x1
                st['b', c] = _stats(x1)
                return tokst(st['b', c][1])
            return Item(0, 75, LAT_X if c == nc - 1 else 0, fn, 2.5)

        def sc(c):
            def fn(tok):
                m, rs_ = st['b', c]
                xn = _pk((Xo[rowsz(c), :] - m) * rs_)
                XN[par][0, c * RC // 2:(c + 1) * RC // 2, :] = xn
                return tokof(xn)
            return Item(0, 22.5, 0, fn, 2.5)
        return [f(c) for f in (sa, sb) for c in range(nc)], [sc(c) for c in range(nc)]

    def d1_streams(r):
        ab, c_ = ln_items(r, lambda c, rs: qb[rs, :].astype(F32), X1, 0)
        for it in c_:
            it.after = 1
        return [proj_items(jnp.maximum(r - 1, 0), Q1, 0) + c_, ab]

    def wprep_items(n):
        ns = pl.ds(_mo(n * 128, 128), 128)

        def f1(tok):
            wqp[:, ns] = pltpu.bitcast(wqkv[:, ns], U32)

        def f2(tok):
            wktp[pl.ds(_mo(n * 64, 64), 64), :] = pltpu.bitcast(wqkv[:, pl.ds(_mo(D + n * 128, 128), 128)].T, U32)
        return [Item(0, 40, 0, f1), Item(0, 200, 0, f2)]

    rr = lax.broadcasted_iota(jnp.int32, (128, 128), 0) // DH
    cc = lax.broadcasted_iota(jnp.int32, (128, 128), 1) // DH
    mask = rr == cc

    def finish_items():
        st = {}

        def fkv(g):
            def fn(tok):
                sl = slice(g * 128, (g + 1) * 128)
                kvg = _nn(P[sl, :].astype(BF16), wqkv[:, 2 * D + g * 128:2 * D + (g + 1) * 128])
                st[g] = jnp.where(mask, kvg, 0.0).astype(BF16)
                P[sl, :] = jnp.zeros((128, D), F32)
            return Item(128, 150, 0, fn)

        def fz(g):
            def fn(tok):
                sl = slice(g * 128, (g + 1) * 128)
                z = jnp.sum(ZP[sl, :], axis=-1, keepdims=True)
                Zm[g] = _pk(jnp.where(mask, jnp.broadcast_to(z, (128, 128)), 0.0))
                ZP[sl, :] = jnp.zeros((128, 128), F32)
            return Item(0, 60, 0, fn)

        def fm(g):
            def fn(tok):
                Mp[g * 64:(g + 1) * 64, :] = _pk(_nn(st[g], wo[g * 128:(g + 1) * 128, :]))
            return Item(128, 80, 0, fn)
        return [f(g) for f in (fkv, fz, fm) for g in range(4)]

    def attn_items(r, Qi, par, sink):
        r0h = _mo(r * 64, 64)
        pn = PN[par]

        def e1(g):
            def fn(tok):
                sl = slice(g * 128, (g + 1) * 128)
                pq = _phi(_bf(_gate(Qi[pl.ds(r0h, 64), sl], tok)).astype(F32))
                den = _nn(pq.astype(BF16), _bf(Zm[g])) + 1e-6
                pn[0, :, sl] = _pk(pq * pl.reciprocal(den, approx=True))
            return Item(32, 150, LAT_M if g == 3 else 0, fn, 3)

        def e3(n):
            def fn(tok):
                sink(n, _nn(_bf(_gate(pn[zi], tok)), _bf(Mp[:, n * 128:(n + 1) * 128])))
            return Item(128, 70, LAT_M if n == 3 else 0, fn, 3)
        return [e1(g) for g in range(4)] + [e3(n) for n in range(4)]

    def att2_items(r, par):
        def sink(n, val):
            ns = slice(n * 128, (n + 1) * 128)
            OO[par][0, :, ns] = val + X1[pl.ds(_mo(r * T, T), T), ns]
        return attn_items(r, Q1, par, sink)

    def ln2_items(r, par):
        ab, c_ = ln_items(r, lambda c, rs: OO[par][zi, c * RC:(c + 1) * RC, :], X3, par)
        return ab + c_

    def att3_items(r, par):
        r0 = _mo(r * T, T)

        def sink(n, val):
            ns = slice(n * 128, (n + 1) * 128)
            ob[pl.ds(r0, T), ns] = (val + X3[pl.ds(r0, T), ns]).astype(BF16)
        return attn_items(r, Q2, par, sink)

    wait(*cp_small)

    def bpre(j, _):
        wait(*cp0(j))
        _merge(pre_items(0, j))
        return 0
    lax.fori_loop(0, NT, bpre, 0)
    start(cp_w, cp_q(0), *cp_sb(2))

    for g in range(NG + 1):
        if g + 1 < NG:
            wait(*cp_sb(g + 1))
        if g >= 1:
            wait(cp_q(g - 1))
        if g == 1:
            start(cp_q(1), *cp_sb(3))
        if g == 2:
            start(cp_q(2), cp_q(3), cp_wv, cp_o)

        def bg(j, _, g=g):
            streams = []
            if g >= 1:
                streams += d1_streams(4 * (g - 1) + j)
            if g + 1 < NG:
                streams.append(pre_items(g + 1, j))
            if g < NG:
                streams.append(mac_items(g, j) + inv_items(g, j))
            _merge(*streams, paced=(0,) if g >= 1 else (), pace=1.1, pin=(1 <= g < NG))
            if g == 0:
                @pl.when(j == 2)
                def _():
                    wait(cp_w)

                @pl.when(j >= 2)
                def _():
                    _merge(wprep_items(2 * (j - 2)), wprep_items(2 * (j - 2) + 1))
            if g == 1:
                @pl.when(j == 0)
                def _():
                    ZP[...] = jnp.zeros(ZP.shape, F32)
            return 0
        lax.fori_loop(0, NT, bg, 0)
    wait(cp_wv, cp_o)
    _merge(proj_items(NB - 1, Q1, 0) + finish_items())

    _merge(att2_items(0, 0))
    _merge(ln2_items(0, 0), att2_items(1, 1))

    def ph2(i, _):
        a = 2 * i
        c = lambda x: jnp.minimum(x, NB - 1)
        _merge(proj_items(a, Q2, 0), ln2_items(a + 1, 1), att2_items(c(a + 2), 0), paced=(0,))
        _merge(proj_items(a + 1, Q2, 1), ln2_items(c(a + 2), 0), att2_items(c(a + 3), 1), paced=(0,))
        return 0
    lax.fori_loop(0, NB // 2, ph2, 0)
    _merge(finish_items())

    def e1s(r, par):
        return att3_items(r, par)[:4]

    def e3s(r, par):
        return att3_items(r, par)[4:]

    _merge(e1s(0, 0), e1s(1, 1))

    def ph3(i, _):
        a = 4 * i
        c = lambda x: jnp.minimum(x, NB - 1)
        _merge(e3s(a, 0), e3s(a + 1, 1), e1s(a + 2, 2), e1s(a + 3, 3))
        start(ocp(a), ocp(a + 1))
        _merge(e3s(a + 2, 2), e3s(a + 3, 3), e1s(c(a + 4), 0), e1s(c(a + 5), 1))
        start(ocp(a + 2), ocp(a + 3))
        return 0
    lax.fori_loop(0, NB // 4, ph3, 0)

    def wt(i, _):
        ocp(i).wait()
        return 0
    lax.fori_loop(0, NB, wt, 0)


@jax.jit
def pallas_interleave_layers__ssm_conv_h3__linear_attn_block__prompt_kernel(
    A_q: jax.Array,
    A_k: jax.Array,
    A_v: jax.Array,
    A_shift_k: jax.Array,
    A_ssm_k: jax.Array,
    A_ssm_D: jax.Array,
    B_x: jax.Array,
    B_wqkv: jax.Array,
    B_wo: jax.Array,
):
    fwd, inv = _dft_mats()
    anyspec = pl.BlockSpec(memory_space=pl.ANY)
    half = lambda r, c: pltpu.VMEM((r // 2, c), U32)
    half1 = lambda r, c: pltpu.VMEM((1, r // 2, c), U32)
    spec = pltpu.VMEM((NT, 4, 3, T, 128), F32)
    out = pl.pallas_call(
        _kernel,
        out_shape=jax.ShapeDtypeStruct((S, D), BF16),
        in_specs=[pl.BlockSpec(memory_space=pltpu.SMEM)] + [anyspec] * 10,
        out_specs=anyspec,
        scratch_shapes=[
            pltpu.VMEM((4, D), BF16),
            pltpu.VMEM((NT, 128), BF16),
            half(2 * T, T), half(T, 2 * T),
            pltpu.VMEM((S, D), BF16),
            pltpu.VMEM((S + HALO, D), BF16),
            pltpu.VMEM((S, D), BF16),
            pltpu.VMEM((D, S), BF16),
            pltpu.VMEM((D, 3 * D), BF16),
            pltpu.VMEM((D, D), BF16),
            half(D, D),
            half(D, D),
            pltpu.VMEM((1, SB + HALO, 128), F32),
            pltpu.VMEM((4, T // 2, 128), U32),
            spec, spec, spec, spec,
            spec, spec, spec, spec,
            pltpu.VMEM((NT, 2, T, 128), F32),
            pltpu.VMEM((NT, T, D), U32),
            pltpu.VMEM((S, D), F32),
            pltpu.VMEM((S, D), F32),
            pltpu.VMEM((S, D), F32),
            half(S, D), half(S, D),
            half1(T, D), half1(T, D),
            half1(D, T), half1(D, T),
            half1(T, D), half1(T, D), half1(T, D), half1(T, D),
            pltpu.VMEM((1, T, D), F32), pltpu.VMEM((1, T, D), F32),
            pltpu.VMEM((D, D), F32),
            pltpu.VMEM((D, 128), F32),
            half(D, D),
            pltpu.VMEM((4, 64, 128), U32),
            pltpu.VMEM((S, D), BF16),
            pltpu.SemaphoreType.DMA((20,)),
            pltpu.SemaphoreType.DMA((NB,)),
            pltpu.SemaphoreType.DMA((3 * NT,)),
        ],
        compiler_params=pltpu.CompilerParams(vmem_limit_bytes=110 * 1024 * 1024),
    )(jnp.zeros((1,), jnp.int32), A_q.reshape(S, D), A_k.reshape(S, D), A_v.reshape(S, D), A_shift_k.T, A_ssm_k,
      A_ssm_D.reshape(NT, 128), B_wqkv, B_wo, jnp.asarray(fwd), jnp.asarray(inv))
    return out.reshape(1, S, D)
```
